```python
import jax
import jax.numpy as jnp

def _softmax(x, axis=-1):
    return jax.nn.softmax(x, axis=axis)
def _gelu(x):
    return jax.nn.gelu(x, approximate=True)
def _silu(x):
    return jax.nn.silu(x)
def _sigmoid(x):
    return jax.nn.sigmoid(x)
def _layernorm(x, axis=-1, eps=1e-5):
    m = jnp.mean(x, axis=axis, keepdims=True)
    v = jnp.var(x, axis=axis, keepdims=True)
    return (x - m) / jnp.sqrt(v + eps)
def _scatter_add(tgt, idx, src, axis=0):
    return tgt.at[idx].add(src)
def _segment_sum(src, seg, n):
    return jax.ops.segment_sum(src, seg, n)
class _Rng:
    def __init__(self, key):
        self._k = key
    def _next(self):
        self._k, sub = jax.random.split(self._k)
        return sub
    def normal(self, shape):
        return jax.random.normal(self._next(), shape, dtype=jnp.bfloat16)
    def randint(self, lo, hi, shape):
        return jax.random.randint(self._next(), shape, lo, hi, dtype=jnp.int32)
    def uniform(self, shape, lo=0.0, hi=1.0):
        return jax.random.uniform(self._next(), shape, jnp.bfloat16, lo, hi)
    def permutation(self, n):
        return jax.random.permutation(self._next(), n)


kernel_name = 'interleave_layers__sliding_local_dilated__glu_gated_swiglu__prompt'

def setup_inputs():
    _rng = _Rng(jax.random.key(int.from_bytes(__import__("os").urandom(4), "little")))
    _w = (lambda a: (lambda t: t.astype(jnp.bfloat16) if jnp.issubdtype(t.dtype, jnp.floating) else t)(jnp.asarray(a)))
    def _A_setup():
        B, S, D = 1, 2048, 1024
        return {
            "x": _w((lambda *s: _rng.normal(s) * 0.05)(B, S, D)),
            "wqkv": _w((lambda *s: _rng.normal(s) * 0.05)(D, 3 * D)),
            "wo": _w((lambda *s: _rng.normal(s) * 0.05)(D, D)),
        }
    _A_in = _A_setup()

    def _B_setup():
        B, S, D, F = 1, 2048, 1024, 3584
        return {
            "x": _w((lambda *s: _rng.normal(s) * 0.05)(B, S, D)),
            "w1": _w((lambda *s: _rng.normal(s) * 0.05)(D, F) * (2.0 / D) ** 0.5),
            "w3": _w((lambda *s: _rng.normal(s) * 0.05)(D, F) * (2.0 / D) ** 0.5),
            "w2": _w((lambda *s: _rng.normal(s) * 0.05)(F, D) * (2.0 / F) ** 0.5),
        }
    _B_in = _B_setup()

    return {
        "A_x": _A_in["x"],
        "A_wqkv": _A_in["wqkv"],
        "A_wo": _A_in["wo"],
        "B_x": _B_in["x"],
        "B_w1": _B_in["w1"],
        "B_w3": _B_in["w3"],
        "B_w2": _B_in["w2"],
    }

def reference(A_x, A_wqkv, A_wo, B_x, B_w1, B_w3, B_w2):
    def _A_ref(x, wqkv, wo):
        B, S, D = x.shape
        H = 32; Dh = D // H
        W, dil = 8, 2
        qkv = (lambda x, *d: x.transpose(*d))((x @ wqkv).reshape(B, S, 3, H, Dh), 2, 0, 3, 1, 4)
        q, k, v = qkv[0], qkv[1], qkv[2]
        scale = Dh ** -0.5
        pos = jnp.arange(S)
        off = jnp.arange(W) * dil
        idx = pos[:, None] - off[None, :]
        mask = idx >= 0
        idx_c = jnp.where(mask, idx, 0).reshape(-1)
        kg = k[:, :, idx_c, :].reshape(B, H, S, W, Dh)
        vg = v[:, :, idx_c, :].reshape(B, H, S, W, Dh)
        logits = jnp.einsum("bhsd,bhswd->bhsw", q, kg) * scale
        logits = jnp.where(mask[None, None, :, :], logits, -1e9)
        attn = _softmax(logits, axis=-1)
        o = jnp.einsum("bhsw,bhswd->bhsd", attn, vg)
        return (lambda x, *d: x.transpose(*d))(o, 0, 2, 1, 3).reshape(B, S, D) @ wo

    def _B_ref(x, w1, w3, w2):
        gate = jnp.einsum("bsd,df->bsf", x, w1)
        up = jnp.einsum("bsd,df->bsf", x, w3)
        h = _silu(gate) * up
        out = jnp.einsum("bsf,fd->bsd", h, w2)
        return out

    x = A_x
    x = x + _A_ref(_layernorm(x, axis=-1), A_wqkv, A_wo)
    x = x + _B_ref(_layernorm(x, axis=-1), B_w1, B_w3, B_w2)
    x = x + _A_ref(_layernorm(x, axis=-1), A_wqkv, A_wo)
    x = x + _B_ref(_layernorm(x, axis=-1), B_w1, B_w3, B_w2)
    return x
```

```python
import functools
import jax
import jax.numpy as jnp
from jax import lax
import jax.experimental.pallas as pl
import jax.experimental.pallas.tpu as pltpu

H, DH, W, DIL = 32, 32, 8, 2
HALO = 16
EPS = 1e-5
F32, BF16 = jnp.float32, jnp.bfloat16


def _ln(x):
    m = jnp.mean(x, axis=-1, keepdims=True)
    c = x - m
    v = jnp.mean(c * c, axis=-1, keepdims=True)
    return c * lax.rsqrt(v + EPS)


def _kernel(x_ref, wqkv_hbm, wo_hbm, w1_hbm, w3_hbm, w2_hbm, o_ref,
            wqkv_raw, wqkv_p, wo_raw, wo_p, w1_v, w3_v, w2_v, tr_scr,
            xs, xn, q_scr, k_scr, v_scr, halo_k, halo_v, a_scr, h_scr, sems, *, T, R, FC):
    D = 1024
    F = w1_v.shape[1]
    step = pl.program_id(0)
    cps = [pltpu.make_async_copy(s, d, sems.at[i]) for i, (s, d) in enumerate(
        [(wqkv_hbm, wqkv_raw), (wo_hbm, wo_raw), (w1_hbm, w1_v), (w3_hbm, w3_v), (w2_hbm, w2_v)])]

    @pl.when(step == 0)
    def _():
        for c in cps:
            c.start()
        halo_k[...] = jnp.zeros_like(halo_k)
        halo_v[...] = jnp.zeros_like(halo_v)
        cps[0].wait()
        for m in range(3):
            for kt in range(4):
                blk = pltpu.bitcast(wqkv_raw[kt * 256:(kt + 1) * 256, m * D:(m + 1) * D], jnp.uint32)
                tr_scr[0] = blk.T
                rows = [tr_scr[0, pl.ds(d, H, stride=DH), :] for d in range(DH)]
                pt = jnp.concatenate(rows, axis=0)
                wqkv_p[kt * 256:(kt + 1) * 256, m * D:(m + 1) * D] = pltpu.bitcast(pt.T, BF16)
        cps[1].wait()
        for c in range(8):
            tr_scr[0] = pltpu.bitcast(wo_raw[:, c * 128:(c + 1) * 128].astype(F32), jnp.uint32)
            rows = [tr_scr[0, pl.ds(d, H, stride=DH), :] for d in range(DH)]
            wo_p[:, c * 128:(c + 1) * 128] = pltpu.bitcast(jnp.concatenate(rows, axis=0), F32).astype(BF16)

    xs[...] = x_ref[...].astype(F32)

    def layer(l, carry):
        xn[...] = _ln(xs[...]).astype(BF16)
        k_scr[:, 0:HALO, :] = halo_k[l]
        v_scr[:, 0:HALO, :] = halo_v[l]
        xv = xn[...]
        q = jnp.dot(xv, wqkv_p[:, 0:D], preferred_element_type=F32) * (DH ** -0.5)
        for j in range(8):
            q_scr[j] = q[:, j * 128:(j + 1) * 128]
        k = jnp.dot(xv, wqkv_p[:, D:2 * D], preferred_element_type=F32)
        for j in range(8):
            k_scr[j, HALO:, :] = k[:, j * 128:(j + 1) * 128]
        v = jnp.dot(xv, wqkv_p[:, 2 * D:3 * D], preferred_element_type=F32)
        for j in range(8):
            v_scr[j, HALO:, :] = v[:, j * 128:(j + 1) * 128]
        halo_k[l] = k_scr[:, T:T + HALO, :]
        halo_v[l] = v_scr[:, T:T + HALO, :]
        for r in range(T // R):
            b = r * R
            ps = []
            for w in range(W):
                p = None
                for j in range(8):
                    t = q_scr[j, b:b + R, :] * k_scr[j, HALO + b - DIL * w:HALO + b - DIL * w + R, :]
                    p = t if p is None else p + t
                p = p + pltpu.roll(p, 64, 1)
                p = p + pltpu.roll(p, 32, 1)
                if b < DIL * w:
                    pos = step * T + b + lax.broadcasted_iota(jnp.int32, (R, 128), 0)
                    p = jnp.where(pos >= DIL * w, p, -1e9)
                ps.append(p)
            mx = functools.reduce(jnp.maximum, ps)
            es = [jnp.exp(p - mx) for p in ps]
            inv = 1.0 / functools.reduce(lambda a, c: a + c, es)
            es = [e * inv for e in es]
            for j in range(8):
                o = None
                for w in range(W):
                    t = es[w] * v_scr[j, HALO + b - DIL * w:HALO + b - DIL * w + R, :]
                    o = t if o is None else o + t
                a_scr[b:b + R, j * 128:(j + 1) * 128] = o.astype(BF16)
        x1 = xs[...] + jnp.dot(a_scr[...], wo_p[...], preferred_element_type=F32)
        xs[...] = x1
        xn[...] = _ln(x1).astype(BF16)

        @pl.when((step == 0) & (l == 0))
        def _():
            cps[2].wait()
            cps[3].wait()
            cps[4].wait()

        xv = xn[...]
        for c in range(F // FC):
            g = jnp.dot(xv, w1_v[:, c * FC:(c + 1) * FC], preferred_element_type=F32)
            u = jnp.dot(xv, w3_v[:, c * FC:(c + 1) * FC], preferred_element_type=F32)
            h_scr[:, c * FC:(c + 1) * FC] = (g * jax.nn.sigmoid(g) * u).astype(BF16)
        xs[...] = xs[...] + jnp.dot(h_scr[...], w2_v[...], preferred_element_type=F32)
        return carry

    lax.fori_loop(0, 2, layer, 0)
    o_ref[...] = xs[...].astype(o_ref.dtype)


def _build(A_x, A_wqkv, A_wo, B_x, B_w1, B_w3, B_w2, T=512, R=16, FC=512):
    del B_x
    B, S, D = A_x.shape
    F = B_w1.shape[1]
    x = A_x.reshape(S, D)
    anyspec = pl.BlockSpec(memory_space=pl.ANY)
    out = pl.pallas_call(
        functools.partial(_kernel, T=T, R=R, FC=FC),
        grid=(S // T,),
        in_specs=[pl.BlockSpec((T, D), lambda i: (i, 0))] + [anyspec] * 5,
        out_specs=pl.BlockSpec((T, D), lambda i: (i, 0)),
        out_shape=jax.ShapeDtypeStruct((S, D), A_x.dtype),
        scratch_shapes=[
            pltpu.VMEM((D, 3 * D), BF16), pltpu.VMEM((D, 3 * D), BF16),
            pltpu.VMEM((D, D), BF16), pltpu.VMEM((D, D), BF16),
            pltpu.VMEM((D, F), BF16), pltpu.VMEM((D, F), BF16), pltpu.VMEM((F, D), BF16),
            pltpu.VMEM((1, D, 128), jnp.uint32),
            pltpu.VMEM((T, D), F32), pltpu.VMEM((T, D), BF16),
            pltpu.VMEM((8, T, 128), F32), pltpu.VMEM((8, T + HALO, 128), F32), pltpu.VMEM((8, T + HALO, 128), F32),
            pltpu.VMEM((2, 8, HALO, 128), F32), pltpu.VMEM((2, 8, HALO, 128), F32),
            pltpu.VMEM((T, D), BF16), pltpu.VMEM((T, F), BF16),
            pltpu.SemaphoreType.DMA((5,)),
        ],
        compiler_params=pltpu.CompilerParams(
            dimension_semantics=("arbitrary",), vmem_limit_bytes=110 * 1024 * 1024),
    )(x, A_wqkv, A_wo, B_w1, B_w3, B_w2)
    return out.reshape(B, S, D)


@jax.jit
def pallas_interleave_layers__sliding_local_dilated__glu_gated_swiglu__prompt_kernel(
        A_x, A_wqkv, A_wo, B_x, B_w1, B_w3, B_w2):
    return _build(A_x, A_wqkv, A_wo, B_x, B_w1, B_w3, B_w2)
```

```python
import contextlib
import functools
import math
import jax
import jax.numpy as jnp
from jax import lax
import jax.experimental.pallas as pl
import jax.experimental.pallas.tpu as pltpu

H, DH, W, DIL = 32, 32, 8, 2
HALO = 16
PAD = DH + 1
EPS = 1e-5
LOG2E = math.log2(math.e)
F32, BF16, U32 = jnp.float32, jnp.bfloat16, jnp.uint32


def _ln(x):
    m = jnp.mean(x, axis=-1, keepdims=True)
    c = x - m
    v = jnp.mean(c * c, axis=-1, keepdims=True)
    return c * lax.rsqrt(v + EPS)


def _dot(a, b):
    return jnp.dot(a, b, preferred_element_type=F32)


def _merge(main, *sides):
    n = len(main)
    for i, f in enumerate(main):
        f()
        for s in sides:
            for g in s[len(s) * i // n:len(s) * (i + 1) // n]:
                g()


def _kernel(x_hbm, wqkv_hbm, wo_hbm, w1_hbm, w3_hbm, w2_hbm, o_hbm,
            wqkv_raw, wqkv_p, wo_raw, wo_p, w1_v, w3_v, w2_v, tr_scr, q_scr, k_scr,
            v_scr, a_scr, xs, xn, io, h_scr, sem_x, sem_w, sem_o, flag, *,
            R, RP, FC, NQ, RL, VS, PM, PN, PMV, PNV, scopes, hack):
    NB = len(xs)
    MB, D = xs[0].shape
    S = NB * MB
    NC = w1_v.shape[0]
    P = functools.partial
    st = contextlib.ExitStack()

    def mark(name):
        st.close()
        if scopes and name:
            st.enter_context(jax.named_scope(name))

    cp_x = [pltpu.make_async_copy(x_hbm.at[r * MB:(r + 1) * MB, :], io[r], sem_x.at[r]) for r in range(NB)]
    cp_out = [pltpu.make_async_copy(io[r], o_hbm.at[r * MB:(r + 1) * MB, :], sem_o.at[r]) for r in range(NB)]
    cp_wq = [pltpu.make_async_copy(wqkv_hbm.at[t * 256:(t + 1) * 256, 0:D],
                                   wqkv_raw.at[0, t * 256:(t + 1) * 256, :], sem_w.at[t]) for t in range(4)]
    cp_wk, cp_wv = [pltpu.make_async_copy(wqkv_hbm.at[:, m * D:(m + 1) * D], wqkv_raw.at[m], sem_w.at[3 + m])
                    for m in (1, 2)]
    cp_wo = pltpu.make_async_copy(wo_hbm, wo_raw, sem_w.at[6])
    cp_ffn = []
    for c in range(NC):
        cp_ffn.append(pltpu.make_async_copy(w1_hbm.at[:, c * FC:(c + 1) * FC], w1_v.at[c], sem_w.at[7]))
        cp_ffn.append(pltpu.make_async_copy(w3_hbm.at[:, c * FC:(c + 1) * FC], w3_v.at[c], sem_w.at[7]))
        cp_ffn.append(pltpu.make_async_copy(w2_hbm.at[c * FC:(c + 1) * FC, :], w2_v.at[c], sem_w.at[7]))

    def stage(slot, i, val):
        for hh in range(4):
            h = 4 * i + hh
            tr_scr[slot][h * PAD:h * PAD + DH, :] = val[hh * DH:(hh + 1) * DH, :]

    def gather(slot, j):
        return jnp.concatenate([tr_scr[slot][pl.ds(4 * j + dd, H, stride=PAD), :] for dd in range(4)], axis=0)

    def qkv_in(m, t, i):
        blk = pltpu.bitcast(wqkv_raw[m, t * 256:(t + 1) * 256, i * 128:(i + 1) * 128], U32)
        stage(t % 2, i, blk.T)

    def qkv_out(m, t, j):
        wqkv_p[m][t * 256:(t + 1) * 256, j * 128:(j + 1) * 128] = pltpu.bitcast(gather(t % 2, j).T, BF16)

    def permute_qkv_steps(m, ts=range(4)):
        return [P(f, m, t, i) for t in ts for f in (qkv_in, qkv_out) for i in range(8)]

    def wo_in(c, i):
        stage(c % 2, i, pltpu.bitcast(wo_raw[i * 128:(i + 1) * 128, c * 128:(c + 1) * 128].astype(F32), U32))

    def wo_out(c, j):
        wo_p[j * 128:(j + 1) * 128, c * 128:(c + 1) * 128] = pltpu.bitcast(gather(c % 2, j), F32).astype(BF16)

    def permute_wo_steps():
        return [P(f, c, i) for c in range(8) for f in (wo_in, wo_out) for i in range(8)]

    def proj(m, r, i, pm, n0, pn):
        y = _dot(xn[r][i:i + pm, :], wqkv_p[m][:, n0:n0 + pn])
        if m == 0:
            y = y * (DH ** -0.5 * LOG2E)
        b = r * MB + i
        for j in range(n0 // 128, (n0 + pn) // 128):
            yj = y[:, j * 128 - n0:(j + 1) * 128 - n0]
            if m == 0:
                q_scr[j, b:b + pm, :] = yj
            elif m == 1:
                k_scr[j, HALO + b:HALO + b + pm, :] = yj
            else:
                v_scr[j][HALO + b:HALO + b + pm, :] = yj
                if b == 0:
                    v_scr[j][0:HALO, :] = jnp.broadcast_to(yj[0:1, :], (HALO, 128))

    def proj_steps(m, rs, n0=0, n1=D, pm=PM, pn=PN):
        return [P(proj, m, r, i, pm, n, pn) for n in range(n0, n1, pn) for r in rs for i in range(0, MB, pm)]

    def probs_steps():
        state = {}

        def step(i):
            b = i * R
            if b < S:
                ps = []
                for w in range(W):
                    p = None
                    for j in range(8):
                        t = q_scr[j, b:b + R, :] * k_scr[j, HALO + b - DIL * w:HALO + b - DIL * w + R, :]
                        p = t if p is None else p + t
                    ps.append(p)
                pp = jnp.concatenate(ps, axis=0)
                state[i] = (pp, pltpu.roll(pp, 64, 1))
            if 0 <= i - 1 < S // R:
                a, c = state[i - 1]
                a = a + c
                state[i - 1] = (a, pltpu.roll(a, 32, 1))
            if i >= 2:
                a, c = state.pop(i - 2)
                a = a + c
                b = (i - 2) * R
                ps = []
                for w in range(W):
                    p = a[w * R:(w + 1) * R]
                    if b < DIL * w:
                        pos = b + lax.broadcasted_iota(jnp.int32, (R, 128), 0)
                        p = jnp.where(pos >= DIL * w, p, -1e9 * LOG2E)
                    ps.append(p)
                mx = functools.reduce(jnp.maximum, ps)
                es = [jnp.exp2(p - mx) for p in ps]
                inv = 1.0 / functools.reduce(lambda u, v: u + v, es)
                for w in range(W):
                    q_scr[w, b:b + R, :] = es[w] * inv
        return [P(step, i) for i in range(S // R + 2)]

    def pv(half, b):
        es = [q_scr[w, b:b + RP, :] for w in range(W)]
        for jj in range(4):
            o = None
            for w in range(W):
                v0 = HALO + b - DIL * w if not hack else max(0, HALO + b - 8 * w)
                t = es[w] * v_scr[4 * half + jj][v0:v0 + RP, :]
                o = t if o is None else o + t
            a_scr[half][b:b + RP, jj * 128:(jj + 1) * 128] = o.astype(BF16)

    def pv_steps(half):
        return [P(pv, half, b) for b in range(0, S, RP)]

    def ln_blk(r, b, load_in, norm, stage_out):
        if load_in:
            xv = io[r][b:b + RL, :].astype(F32)
            xs[r][b:b + RL, :] = xv
        else:
            xv = xs[r][b:b + RL, :]
        if norm:
            xn[r][b:b + RL, :] = _ln(xv).astype(BF16)
        if stage_out:
            io[r][b:b + RL, :] = xv.astype(BF16)

    def ln_steps(r, load_in=False, norm=True, stage_out=False):
        return [P(ln_blk, r, b, load_in, norm, stage_out) for b in range(0, MB, RL)]

    def wo_mm(half, r, i, n):
        xs[r][i:i + PM, n:n + PN] += _dot(a_scr[half][r * MB + i:r * MB + i + PM, :],
                                          wo_p[half * (D // 2):(half + 1) * (D // 2), n:n + PN])

    def wo_steps(half, rs):
        return [P(wo_mm, half, r, i, n) for r in rs for n in range(0, D, PN) for i in range(0, MB, PM)]

    def ffn_up(c, r, i=0, pm=MB, n=0, pn=FC):
        g = _dot(xn[r][i:i + pm, :], w1_v[c, :, n:n + pn])
        u = _dot(xn[r][i:i + pm, :], w3_v[c, :, n:n + pn])
        h_scr[r][i:i + pm, n:n + pn] = (g * jax.nn.sigmoid(g) * u).astype(BF16)

    def up_steps(c, r, pm=MB, pn=FC):
        return [P(ffn_up, c, r, i, pm, n, pn) for n in range(0, FC, pn) for i in range(0, MB, pm)]

    def ffn_down(c, r, i, pm, n, pn):
        xs[r][i:i + pm, n:n + pn] += _dot(h_scr[r][i:i + pm, :], w2_v[c, :, n:n + pn])

    def down_steps(c, r, pm=MB, pn=NQ):
        return [P(ffn_down, c, r, i, pm, n, pn) for n in range(0, D, pn) for i in range(0, MB, pm)]

    mark('pro')
    flag[0] = 1
    cp_x[0].start()
    for c in cp_wq:
        c.start()
    for c in cp_x[1:]:
        c.start()
    k_scr[:, 0:HALO, :] = jnp.zeros((8, HALO, 128), F32)
    cp_x[0].wait()
    _merge(ln_steps(0, load_in=True))
    for t in range(4):
        cp_wq[t].wait()
        _merge(permute_qkv_steps(0, [t]))
    cp_wk.start()
    cp_wv.start()
    cp_wo.start()
    mark(None)

    def phase(name):
        def deco(fn):
            mark(name)
            pl.when(flag[0] == 1)(fn)
            mark(None)
        return deco

    def layer(l):
        if l == 0:
            pk = permute_qkv_steps(1)
            for r in range(NB):
                if r + 1 < NB:
                    cp_x[r + 1].wait()
                else:
                    cp_wk.wait()

                @phase('Q')
                def _():
                    _merge(proj_steps(0, [r]), ln_steps(r + 1, load_in=True) if r + 1 < NB else pk)
            cp_wv.wait()
            cp_wo.wait()
            for c in cp_ffn:
                c.start()

            @phase('K')
            def _():
                _merge(proj_steps(1, range(NB)), permute_qkv_steps(2) + permute_wo_steps())
        else:
            @phase('QK')
            def _():
                _merge(proj_steps(0, [0]), ln_steps(NB - 1))
                _merge(proj_steps(0, range(1, NB), pm=MB, pn=NQ))
                _merge(proj_steps(1, range(NB), pm=MB, pn=NQ))

        @phase('V0')
        def _():
            _merge(proj_steps(2, range(NB), 0, VS, PMV, PNV), probs_steps())

        @phase('V1')
        def _():
            _merge(proj_steps(2, range(NB), VS, D), pv_steps(0))

        @phase('WO0')
        def _():
            _merge(wo_steps(0, range(NB)), pv_steps(1))

        if l == 0:
            for c in cp_ffn:
                c.wait()

        @phase('WO1')
        def _():
            for r in range(NB):
                _merge(wo_steps(1, [r]), ln_steps(r - 1) if r else [])

        @phase('F0')
        def _():
            for r in range(NB):
                _merge(up_steps(0, r) if r else up_steps(0, r, PM, PN), [] if r else ln_steps(NB - 1))
            for r in range(NB):
                _merge(down_steps(0, r))

        mark('Floop')

        def chunk(c, carry):
            for r in range(NB):
                ffn_up(c, r)
            for r in range(NB):
                _merge(down_steps(c, r))
            return carry
        lax.fori_loop(1, NC - 1, chunk, 0)

        @phase('Flast')
        def _():
            for r in range(NB):
                ffn_up(NC - 1, r)
            for r in range(NB):
                _merge(down_steps(NC - 1, r, PM, 256) if r else down_steps(NC - 1, r),
                       ln_steps(r - 1, norm=not l, stage_out=l) if r else [])
                if r and l:
                    cp_out[r - 1].start()
            if l:
                _merge(ln_steps(NB - 1, norm=False, stage_out=True))
                cp_out[NB - 1].start()

    layer(0)
    layer(1)
    for c in cp_out:
        c.wait()


def _build(A_x, A_wqkv, A_wo, B_x, B_w1, B_w3, B_w2, R=8, RP=16, FC=256, NQ=256, NB=4, RL=64,
           VS=768, PM=128, PN=128, PMV=256, PNV=256, scopes=False, hack=0):
    del B_x
    B, S, D = A_x.shape
    F = B_w1.shape[1]
    NC = F // FC
    MB = S // NB
    x = A_x.reshape(S, D)
    anyspec = pl.BlockSpec(memory_space=pl.ANY)
    out = pl.pallas_call(
        functools.partial(_kernel, R=R, RP=RP, FC=FC, NQ=NQ, RL=RL, VS=VS, scopes=scopes, hack=hack, PM=PM, PN=PN, PMV=PMV, PNV=PNV),
        in_specs=[anyspec] * 6,
        out_specs=anyspec,
        out_shape=jax.ShapeDtypeStruct((S, D), A_x.dtype),
        scratch_shapes=[
            pltpu.VMEM((3, D, D), BF16), [pltpu.VMEM((D, D), BF16)] * 3,
            pltpu.VMEM((D, D), BF16), pltpu.VMEM((D, D), BF16),
            pltpu.VMEM((NC, D, FC), BF16), pltpu.VMEM((NC, D, FC), BF16), pltpu.VMEM((NC, FC, D), BF16),
            [pltpu.VMEM((H * PAD, 128), U32)] * 2,
            pltpu.VMEM((8, S, 128), F32), pltpu.VMEM((8, S + HALO, 128), F32),
            [pltpu.VMEM((S + HALO, 128), F32)] * 8,
            [pltpu.VMEM((S, D // 2), BF16)] * 2,
            [pltpu.VMEM((MB, D), F32)] * NB, [pltpu.VMEM((MB, D), BF16)] * NB, [pltpu.VMEM((MB, D), BF16)] * NB,
            [pltpu.VMEM((MB, FC), BF16)] * NB,
            pltpu.SemaphoreType.DMA((NB,)), pltpu.SemaphoreType.DMA((8,)), pltpu.SemaphoreType.DMA((NB,)),
            pltpu.SMEM((1,), jnp.int32),
        ],
        compiler_params=pltpu.CompilerParams(vmem_limit_bytes=120 * 1024 * 1024),
    )(x, A_wqkv, A_wo, B_w1, B_w3, B_w2)
    return out.reshape(B, S, D)


@jax.jit
def pallas_interleave_layers__sliding_local_dilated__glu_gated_swiglu__prompt_kernel(
        A_x, A_wqkv, A_wo, B_x, B_w1, B_w3, B_w2):
    return _build(A_x, A_wqkv, A_wo, B_x, B_w1, B_w3, B_w2)
```

```python
import contextlib
import functools
import math
import jax
import jax.numpy as jnp
from jax import lax
import jax.experimental.pallas as pl
import jax.experimental.pallas.tpu as pltpu

H, DH, W, DIL = 32, 32, 8, 2
HALO = 16
PAD = DH + 1
EPS = 1e-5
LOG2E = math.log2(math.e)
F32, BF16, U32 = jnp.float32, jnp.bfloat16, jnp.uint32


def _ln(x):
    m = jnp.mean(x, axis=-1, keepdims=True)
    c = x - m
    v = jnp.mean(c * c, axis=-1, keepdims=True)
    return c * lax.rsqrt(v + EPS)


def _dot(a, b):
    return jnp.dot(a, b, preferred_element_type=F32)


def _merge(main, *sides):
    n = len(main)
    for i, f in enumerate(main):
        f()
        for s in sides:
            for g in s[len(s) * i // n:len(s) * (i + 1) // n]:
                g()


def _kernel(x_hbm, wqkv_hbm, wo_hbm, w1_hbm, w3_hbm, w2_hbm, o_hbm,
            wqkv_raw, wqkv_p, wo_raw, wo_p, w1_v, w3_v, w2_v, tr_scr, q_scr, k_scr,
            v_scr, a_scr, xs, xn, io, h_scr, sem_x, sem_w, sem_o, flag, *,
            R, RP, FC, NQ, RL, JP, BAR, PM, PN, PMV, PNV, PMP, PNP, PMO, PNO, PML, PNL, OB, CH, QS, PND, scopes):
    NB = len(xs)
    MB, D = xs[0].shape
    S = NB * MB
    NC = w1_v.shape[0]
    P = functools.partial
    st = contextlib.ExitStack()

    def mark(name):
        st.close()
        if scopes and name:
            st.enter_context(jax.named_scope(name))

    cp_x = [pltpu.make_async_copy(x_hbm.at[r * MB:(r + 1) * MB, :], io[r], sem_x.at[r]) for r in range(NB)]

    def cp_out(r, i, n):
        return pltpu.make_async_copy(io[r].at[i:i + n, :], o_hbm.at[r * MB + i:r * MB + i + n, :], sem_o.at[r])

    cp_wq = [pltpu.make_async_copy(wqkv_hbm.at[t * 256:(t + 1) * 256, 0:D],
                                   wqkv_raw.at[0, t * 256:(t + 1) * 256, :], sem_w.at[t]) for t in range(4)]
    cp_wk, cp_wv = [pltpu.make_async_copy(wqkv_hbm.at[:, m * D:(m + 1) * D], wqkv_raw.at[m], sem_w.at[3 + m])
                    for m in (1, 2)]
    cp_wo = pltpu.make_async_copy(wo_hbm, wo_raw, sem_w.at[6])
    cp_ffn = []
    for c in range(NC):
        cp_ffn.append(pltpu.make_async_copy(w1_hbm.at[:, c * FC:(c + 1) * FC], w1_v.at[c], sem_w.at[7]))
        cp_ffn.append(pltpu.make_async_copy(w3_hbm.at[:, c * FC:(c + 1) * FC], w3_v.at[c], sem_w.at[7]))
        cp_ffn.append(pltpu.make_async_copy(w2_hbm.at[c * FC:(c + 1) * FC, :], w2_v.at[c], sem_w.at[7]))

    def stage(slot, i, val):
        for hh in range(4):
            h = 4 * i + hh
            tr_scr[slot][h * PAD:h * PAD + DH, :] = val[hh * DH:(hh + 1) * DH, :]

    def gather(slot, j):
        return jnp.concatenate([tr_scr[slot][pl.ds(4 * j + dd, H, stride=PAD), :] for dd in range(4)], axis=0)

    def qkv_in(m, t, i):
        blk = pltpu.bitcast(wqkv_raw[m, t * 256:(t + 1) * 256, i * 128:(i + 1) * 128], U32)
        stage(t % 2, i, blk.T)

    def qkv_out(m, t, j):
        wqkv_p[m][t * 256:(t + 1) * 256, j * 128:(j + 1) * 128] = pltpu.bitcast(gather(t % 2, j).T, BF16)

    def permute_qkv_steps(m, ts=range(4)):
        return [P(f, m, t, i) for t in ts for f in (qkv_in, qkv_out) for i in range(8)]

    def wo_in(c, i):
        stage(c % 2, i, pltpu.bitcast(wo_raw[i * 128:(i + 1) * 128, c * 128:(c + 1) * 128].astype(F32), U32))

    def wo_out(c, j):
        wo_p[j * 128:(j + 1) * 128, c * 128:(c + 1) * 128] = pltpu.bitcast(gather(c % 2, j), F32).astype(BF16)

    def permute_wo_steps():
        return [P(f, c, i) for c in range(8) for f in (wo_in, wo_out) for i in range(8)]

    def proj(m, r, i, pm, n0, pn):
        y = _dot(xn[r][i:i + pm, :], wqkv_p[m][:, n0:n0 + pn])
        if m == 0:
            y = y * (DH ** -0.5 * LOG2E)
        b = r * MB + i
        for j in range(n0 // 128, (n0 + pn) // 128):
            yj = y[:, j * 128 - n0:(j + 1) * 128 - n0]
            if m == 0:
                q_scr[j, b:b + pm, :] = yj
            elif m == 1:
                k_scr[j, HALO + b:HALO + b + pm, :] = yj
            else:
                v_scr[j][HALO + b:HALO + b + pm, :] = yj
                if b == 0:
                    v_scr[j][0:HALO, :] = jnp.broadcast_to(yj[0:1, :], (HALO, 128))

    def proj_steps(m, rs, n0=0, n1=D, pm=PM, pn=PN):
        return [P(proj, m, r, i, pm, n, pn) for n in range(n0, n1, pn) for r in rs for i in range(0, MB, pm)]

    def probs_steps(r, half):
        state = {}
        nst = MB // R // 2
        base = r * MB + half * (MB // 2)

        def step(i):
            b = base + i * R
            if i < nst:
                ps = []
                for w in range(W):
                    p = None
                    for j in range(8):
                        t = q_scr[j, b:b + R, :] * k_scr[j, HALO + b - DIL * w:HALO + b - DIL * w + R, :]
                        p = t if p is None else p + t
                    ps.append(p)
                pp = jnp.concatenate(ps, axis=0)
                state[i] = (pp, pltpu.roll(pp, 64, 1))
            if 0 <= i - 1 < nst:
                a, c = state[i - 1]
                a = a + c
                state[i - 1] = (a, pltpu.roll(a, 32, 1))
            if i >= 2:
                a, c = state.pop(i - 2)
                a = a + c
                b = base + (i - 2) * R
                ps = []
                for w in range(W):
                    p = a[w * R:(w + 1) * R]
                    if b < DIL * w:
                        pos = b + lax.broadcasted_iota(jnp.int32, (R, 128), 0)
                        p = jnp.where(pos >= DIL * w, p, -1e9 * LOG2E)
                    ps.append(p)
                mx = functools.reduce(jnp.maximum, ps)
                es = [jnp.exp2(p - mx) for p in ps]
                inv = 1.0 / functools.reduce(lambda u, v: u + v, es)
                for w in range(W):
                    q_scr[w, b:b + R, :] = es[w] * inv
        return [P(step, i) for i in range(nst + 2)]

    def pv(r, i, js):
        b = r * MB + i
        es = [q_scr[w, b:b + RP, :] for w in range(W)]
        for j in js:
            o = None
            for w in range(W):
                t = es[w] * v_scr[j][HALO + b - DIL * w:HALO + b - DIL * w + RP, :]
                o = t if o is None else o + t
            a_scr[r][i:i + RP, j * 128:(j + 1) * 128] = o.astype(BF16)

    def pv_steps(r):
        return [P(pv, r, i, range(j, j + JP)) for i in range(0, MB, RP) for j in range(0, 8, JP)]

    def ln_blk(r, b, load_in, norm, stage_out):
        if load_in:
            xv = io[r][b:b + RL, :].astype(F32)
            xs[r][b:b + RL, :] = xv
        else:
            xv = xs[r][b:b + RL, :]
        if norm:
            xn[r][b:b + RL, :] = _ln(xv).astype(BF16)
        if stage_out:
            io[r][b:b + RL, :] = xv.astype(BF16)

    def ln_steps(r, load_in=False, norm=True, stage_out=False, i0=0, i1=MB):
        return [P(ln_blk, r, b, load_in, norm, stage_out) for b in range(i0, i1, RL)]

    def wo_mm(r, i, n):
        xs[r][i:i + PMO, n:n + PNO] += _dot(a_scr[r][i:i + PMO, :], wo_p[:, n:n + PNO])

    def wo_steps(r, i0=0, i1=MB):
        return [P(wo_mm, r, i, n) for n in range(0, D, PNO) for i in range(i0, i1, PMO)]

    def ffn_up(c, r, i=0, pm=MB, n=0, pn=FC):
        g = _dot(xn[r][i:i + pm, :], w1_v[c, :, n:n + pn])
        u = _dot(xn[r][i:i + pm, :], w3_v[c, :, n:n + pn])
        h_scr[r][i:i + pm, n:n + pn] = (g * jax.nn.sigmoid(g) * u).astype(BF16)

    def up_steps(c, r, pm=MB, pn=FC, i0=0, i1=MB):
        return [P(ffn_up, c, r, i, pm, n, pn) for n in range(0, FC, pn) for i in range(i0, i1, pm)]

    def ffn_down(c, r, i, pm, n, pn):
        xs[r][i:i + pm, n:n + pn] += _dot(h_scr[r][i:i + pm, :], w2_v[c, :, n:n + pn])

    def down_steps(c, r, pm=MB, pn=NQ, i0=0, i1=MB):
        return [P(ffn_down, c, r, i, pm, n, pn) for n in range(0, D, pn) for i in range(i0, i1, pm)]

    mark('pro')
    flag[0] = 1
    for c in cp_wq[:3]:
        c.start()
    k_scr[:, 0:HALO, :] = jnp.zeros((8, HALO, 128), F32)
    prev = []
    for t, nxt in enumerate((cp_wq[3], cp_x[0], cp_wk, cp_wv)):
        cp_wq[t].wait()
        nxt.start()
        steps = permute_qkv_steps(0, [t])
        _merge(steps[:8], prev)
        prev = steps[8:]
    _merge(prev)
    cp_x[0].wait()
    _merge(ln_steps(0, load_in=True, i0=0, i1=CH))
    mark(None)

    def phase(name):
        def deco(fn):
            mark(name)
            pl.when(flag[0] == 1)(fn)
            mark(None)
        return deco

    def layer(l):
        def run(name, main, *sides):
            phase(name)(lambda: _merge(main, *sides))

        def halves(steps):
            return steps[:len(steps) // 2], steps[len(steps) // 2:]

        def first(steps, *waits):
            if l:
                return []
            for c in waits:
                c.wait()
            return steps

        def qkv(m, r):
            return proj_steps(m, [r], 0, D, *((PMP, PNP) if m == 0 or r == 0 else (PMV, PNV)))

        pwo = halves(permute_wo_steps())
        pb = va = vb = []
        for r in range(NB):
            if r == 0:
                if l:
                    run('Q0', qkv(0, r), ln_steps(NB - 1))
                    run('K0', qkv(1, r))
                else:
                    def q0(i, *sides):
                        _merge([P(proj, 0, 0, i, CH, n, 128) for n in range(0, D, 128)],
                               ln_steps(0, load_in=True, i0=i + CH, i1=min(i + 2 * CH, MB)), *sides)
                    phase('Q0a')(lambda: [q0(i) for i in range(0, QS, CH)] and None)
                    cp_wk.wait()
                    for c in [cp_x[1], cp_wo] + cp_x[2:]:
                        c.start()
                    pk = permute_qkv_steps(1)
                    n = (MB - QS) // CH
                    phase('Q0b')(lambda: [q0(QS + u * CH, pk[u * len(pk) // n:(u + 1) * len(pk) // n])
                                          for u in range(n)] and None)
                    run('K0', qkv(1, r), first(permute_qkv_steps(2), cp_wv))
                    for c in cp_ffn:
                        c.start()
            else:
                run('Q%d' % r, qkv(0, r), pb, ln_steps(r - 2) if r > 1 else first(pwo[0], cp_wo))
                run('K%d' % r, qkv(1, r), va, first(pwo[1]) if r == 1 else [])
            pa, pb = probs_steps(r, 0), probs_steps(r, 1)
            nxt = first(ln_steps(r + 1, load_in=True), cp_x[r + 1]) if r + 1 < NB else []
            if r == 0:
                run('V0', qkv(2, r), pa, nxt)
            else:
                run('V%d' % r, qkv(2, r), vb, nxt)
                run('O%d' % (r - 1), wo_steps(r - 1), pa)
            va, vb = halves(pv_steps(r))
        if l == 0:
            for c in cp_ffn:
                c.wait()

        def up(r):
            return up_steps(0, r, PM, PN)

        def down(r):
            return down_steps(0, r, PM, 256)

        run('F0a', up(0) + down(0), pb, ln_steps(NB - 2))
        run('F0b', up_steps(0, 1, PMV, PNV) + down_steps(0, 1, PMV, PND), va)
        run('F0c', up_steps(0, 2, PMV, PNV) + down_steps(0, 2, PMV, PND), vb)
        hb = MB // 2
        run('O3a', wo_steps(3, 0, hb))
        run('O3b', wo_steps(3, hb, MB), ln_steps(3, i0=0, i1=hb))
        run('F0d', up_steps(0, 3, PM, PN, 0, hb), ln_steps(3, i0=hb))
        run('F0e', up_steps(0, 3, hb, FC, hb, MB) + down_steps(0, 3))

        mark('Floop')

        def chunk(c, carry):
            for r in range(NB):
                ffn_up(c, r)
            for r in range(NB):
                _merge(down_steps(c, r))
            return carry
        lax.fori_loop(1, NC - 1, chunk, 0)

        c = NC - 1
        for r in range(NB):
            if l == 0:
                if r:
                    run('L%d' % r, up_steps(c, r, PML, PNL) + down_steps(c, r, PML, 256), ln_steps(r - 1))
                else:
                    run('L0', up_steps(c, r) + down_steps(c, r))
            else:
                @phase('L%d' % r)
                def _():
                    _merge(up_steps(c, r))
                    ob = MB if r + 1 < NB else OB
                    for i in range(0, MB, ob):
                        _merge(down_steps(c, r, ob, NQ, i, i + ob))
                        _merge(ln_steps(r, norm=False, stage_out=True, i0=i, i1=i + ob))
                        cp_out(r, i, ob).start()

    layer(0)
    layer(1)
    for r in range(NB):
        cp_out(r, 0, MB).wait()


def _build(A_x, A_wqkv, A_wo, B_x, B_w1, B_w3, B_w2, R=8, RP=16, FC=256, NQ=256, NB=4, RL=32,
           JP=1, BAR='QKVO', PM=128, PN=128, PMV=128, PNV=128, PMP=256, PNP=128, PMO=256, PNO=128, PML=256, PNL=128, OB=128, CH=128, QS=256, PND=256, scopes=False):
    del B_x
    B, S, D = A_x.shape
    F = B_w1.shape[1]
    NC = F // FC
    MB = S // NB
    x = A_x.reshape(S, D)
    anyspec = pl.BlockSpec(memory_space=pl.ANY)
    out = pl.pallas_call(
        functools.partial(_kernel, R=R, RP=RP, FC=FC, NQ=NQ, RL=RL, JP=JP, BAR=BAR, scopes=scopes, PM=PM, PN=PN, PMV=PMV, PNV=PNV, PMP=PMP, PNP=PNP, PMO=PMO, PNO=PNO, PML=PML, PNL=PNL, OB=OB, CH=CH, QS=QS, PND=PND),
        in_specs=[anyspec] * 6,
        out_specs=anyspec,
        out_shape=jax.ShapeDtypeStruct((S, D), A_x.dtype),
        scratch_shapes=[
            pltpu.VMEM((3, D, D), BF16), [pltpu.VMEM((D, D), BF16)] * 3,
            pltpu.VMEM((D, D), BF16), pltpu.VMEM((D, D), BF16),
            pltpu.VMEM((NC, D, FC), BF16), pltpu.VMEM((NC, D, FC), BF16), pltpu.VMEM((NC, FC, D), BF16),
            [pltpu.VMEM((H * PAD, 128), U32)] * 2,
            pltpu.VMEM((8, S, 128), F32), pltpu.VMEM((8, S + HALO, 128), F32),
            [pltpu.VMEM((S + HALO, 128), F32)] * 8,
            [pltpu.VMEM((MB, D), BF16)] * NB,
            [pltpu.VMEM((MB, D), F32)] * NB, [pltpu.VMEM((MB, D), BF16)] * NB, [pltpu.VMEM((MB, D), BF16)] * NB,
            [pltpu.VMEM((MB, FC), BF16)] * NB,
            pltpu.SemaphoreType.DMA((NB,)), pltpu.SemaphoreType.DMA((8,)), pltpu.SemaphoreType.DMA((NB,)),
            pltpu.SMEM((1,), jnp.int32),
        ],
        compiler_params=pltpu.CompilerParams(vmem_limit_bytes=120 * 1024 * 1024),
    )(x, A_wqkv, A_wo, B_w1, B_w3, B_w2)
    return out.reshape(B, S, D)


@jax.jit
def pallas_interleave_layers__sliding_local_dilated__glu_gated_swiglu__prompt_kernel(
        A_x, A_wqkv, A_wo, B_x, B_w1, B_w3, B_w2):
    return _build(A_x, A_wqkv, A_wo, B_x, B_w1, B_w3, B_w2)
```

```python
import contextlib
import functools
import math
import jax
import jax.numpy as jnp
from jax import lax
import jax.experimental.pallas as pl
import jax.experimental.pallas.tpu as pltpu

H, DH, W, DIL = 32, 32, 8, 2
HALO = 16
PAD = DH + 1
EPS = 1e-5
LOG2E = math.log2(math.e)
F32, BF16, U32 = jnp.float32, jnp.bfloat16, jnp.uint32


def _ln(x):
    m = jnp.mean(x, axis=-1, keepdims=True)
    c = x - m
    v = jnp.mean(c * c, axis=-1, keepdims=True)
    return c * lax.rsqrt(v + EPS)


def _dot(a, b):
    return jnp.dot(a, b, preferred_element_type=F32)


def _ld(ref, r0, r1, cols=slice(None)):
    return pltpu.bitcast(ref[r0 // 2:r1 // 2, cols], BF16)


def _st(ref, r0, val, cols=slice(None)):
    ref[r0 // 2:(r0 + val.shape[0]) // 2, cols] = pltpu.bitcast(val.astype(BF16), U32)


def _merge(main, *sides):
    n = len(main)
    for i, f in enumerate(main):
        f()
        for s in sides:
            for g in s[len(s) * i // n:len(s) * (i + 1) // n]:
                g()


def _kernel(x_hbm, wqkv_hbm, wo_hbm, w1_hbm, w3_hbm, w2_hbm, o_hbm,
            wqkv_raw, wqkv_p, wo_raw, wo_p, w1_v, w3_v, w2_v, tr_scr, q_scr, k_scr,
            v_scr, a_scr, xs, xn, io, h_scr, sem_x, sem_w, sem_o, flag, *,
            R, RP, FC, NQ, RL, JP, BAR, PM, PN, PMV, PNV, PMP, PNP, PMO, PNO, PML, PNL, OB, LD, INF, PMD, PNDU, PND, JOIN, LAYERS, DLY, LNP, scopes):
    NB = len(xs)
    MB, D = xs[0].shape
    S = NB * MB
    NC = w1_v.shape[0]
    P = functools.partial
    st = contextlib.ExitStack()

    def mark(name):
        st.close()
        if scopes and name:
            st.enter_context(jax.named_scope(name))

    cp_x = {r: pltpu.make_async_copy(x_hbm.at[r * MB:(r + 1) * MB, :], io[r], sem_x.at[r]) for r in range(1, NB)}

    def cp_out(r, i, n):
        return pltpu.make_async_copy(io[r].at[i:i + n, :], o_hbm.at[r * MB + i:r * MB + i + n, :], sem_o.at[r])

    cp_wq, cp_wk = [[pltpu.make_async_copy(wqkv_hbm.at[t * 256:(t + 1) * 256, m * D:(m + 1) * D],
                                           wqkv_raw.at[m, t * 256:(t + 1) * 256, :], sem_w.at[4 * m + t])
                     for t in range(4)] for m in range(2)]
    cp_wv = pltpu.make_async_copy(wqkv_hbm.at[:, 2 * D:3 * D], wqkv_raw.at[2], sem_w.at[8])
    HB = MB // 2
    cp_x0 = [pltpu.make_async_copy(x_hbm.at[i * HB:(i + 1) * HB, :], io[0].at[i * HB:(i + 1) * HB, :],
                                   sem_w.at[11 + i]) for i in range(2)]
    cp_wo = pltpu.make_async_copy(wo_hbm, wo_raw, sem_w.at[9])
    cp_ffn = []
    for c in range(NC):
        cp_ffn.append(pltpu.make_async_copy(w1_hbm.at[:, c * FC:(c + 1) * FC], w1_v.at[c], sem_w.at[10]))
        cp_ffn.append(pltpu.make_async_copy(w3_hbm.at[:, c * FC:(c + 1) * FC], w3_v.at[c], sem_w.at[10]))
        cp_ffn.append(pltpu.make_async_copy(w2_hbm.at[c * FC:(c + 1) * FC, :], w2_v.at[c], sem_w.at[10]))

    def stage(slot, i, val):
        for hh in range(4):
            h = 4 * i + hh
            tr_scr[slot][h * PAD:h * PAD + DH, :] = val[hh * DH:(hh + 1) * DH, :]

    def gather(slot, j):
        return jnp.concatenate([tr_scr[slot][pl.ds(4 * j + dd, H, stride=PAD), :] for dd in range(4)], axis=0)

    def qkv_in(m, t, i):
        blk = pltpu.bitcast(wqkv_raw[m, t * 256:(t + 1) * 256, i * 128:(i + 1) * 128], U32)
        stage(t % 2, i, blk.T)

    def qkv_out(m, t, j):
        wqkv_p[m][t * 128:(t + 1) * 128, j * 128:(j + 1) * 128] = gather(t % 2, j).T

    def permute_qkv_steps(m, ts=range(4)):
        return [P(f, m, t, i) for t in ts for f in (qkv_in, qkv_out) for i in range(8)]

    def wo_in(c, i):
        stage(c % 2, i, pltpu.bitcast(wo_raw[i * 128:(i + 1) * 128, c * 128:(c + 1) * 128].astype(F32), U32))

    def wo_out(c, j):
        _st(wo_p, j * 128, pltpu.bitcast(gather(c % 2, j), F32), slice(c * 128, (c + 1) * 128))

    def permute_wo_steps():
        return [P(f, c, i) for c in range(8) for f in (wo_in, wo_out) for i in range(8)]

    def proj(m, r, i, pm, n0, pn):
        y = _dot(_ld(xn[r], i, i + pm), _ld(wqkv_p[m], 0, D, slice(n0, n0 + pn)))
        if m == 0:
            y = y * (DH ** -0.5 * LOG2E)
        b = r * MB + i
        for j in range(n0 // 128, (n0 + pn) // 128):
            yj = y[:, j * 128 - n0:(j + 1) * 128 - n0]
            if m == 0:
                q_scr[j, b:b + pm, :] = yj
            elif m == 1:
                k_scr[j, HALO + b:HALO + b + pm, :] = yj
            else:
                v_scr[j][HALO + b:HALO + b + pm, :] = yj
                if b == 0:
                    v_scr[j][0:HALO, :] = jnp.broadcast_to(yj[0:1, :], (HALO, 128))

    def proj_steps(m, rs, n0=0, n1=D, pm=PM, pn=PN):
        return [P(proj, m, r, i, pm, n, pn) for n in range(n0, n1, pn) for r in rs for i in range(0, MB, pm)]

    def probs_steps(r, half):
        base = r * MB + half * (MB // 2)
        items = [(b, w) for b in range(base, base + MB // 2, R) for w in range(W)]
        s1, s2, done, qs = {}, {}, [], {}

        def step(t):
            if t < len(items):
                b, w = items[t]
                if w == 0:
                    qs[b] = [q_scr[j, b:b + R, :] for j in range(8)]
                p = None
                for j in range(8):
                    u = qs[b][j] * k_scr[j, HALO + b - DIL * w:HALO + b - DIL * w + R, :]
                    p = u if p is None else p + u
                s1[t] = (p, pltpu.roll(p, 64, 1))
            if 0 <= t - DLY < len(items):
                u, v = s1.pop(t - DLY)
                u = u + v
                s2[t - DLY] = (u, pltpu.roll(u, 32, 1))
            if t - 2 * DLY >= 0:
                b, w = items[t - 2 * DLY]
                u, v = s2.pop(t - 2 * DLY)
                p = u + v
                if b < DIL * w:
                    pos = b + lax.broadcasted_iota(jnp.int32, (R, 128), 0)
                    p = jnp.where(pos >= DIL * w, p, -1e9 * LOG2E)
                done.append(p)
                if w == W - 1:
                    mx = functools.reduce(jnp.maximum, done)
                    es = [jnp.exp2(p - mx) for p in done]
                    inv = 1.0 / functools.reduce(lambda u, v: u + v, es)
                    for w in range(W):
                        q_scr[w, b:b + R, :] = es[w] * inv
                    done.clear()
        return [P(step, t) for t in range(len(items) + 2 * DLY)]

    def pv(r, i, js):
        b = r * MB + i
        es = [q_scr[w, b:b + RP, :] for w in range(W)]
        for j in js:
            o = None
            for w in range(W):
                t = es[w] * v_scr[j][HALO + b - DIL * w:HALO + b - DIL * w + RP, :]
                o = t if o is None else o + t
            _st(a_scr[r], i, o, slice(j * 128, (j + 1) * 128))

    def pv_steps(r):
        return [P(pv, r, i, range(j, j + JP)) for i in range(0, MB, RP) for j in range(0, 8, JP)]

    def ln_steps(r, load_in=False, i0=0, i1=MB):
        rows = list(range(i0, i1, RL))
        mean, var = {}, {}

        def step(t):
            if t < len(rows):
                b = rows[t]
                if load_in:
                    x = io[r][b:b + RL, :].astype(F32)
                    xs[r][b:b + RL, :] = x
                else:
                    x = xs[r][b:b + RL, :]
                mean[b] = jnp.mean(x, axis=-1, keepdims=True)
            if 0 <= t - LD < len(rows):
                b = rows[t - LD]
                c = xs[r][b:b + RL, :] - mean[b]
                var[b] = jnp.mean(c * c, axis=-1, keepdims=True)
            if t - 2 * LD >= 0:
                b = rows[t - 2 * LD]
                c = xs[r][b:b + RL, :] - mean.pop(b)
                _st(xn[r], b, c * lax.rsqrt(var.pop(b) + EPS))
        return [P(step, t) for t in range(len(rows) + 2 * LD)]

    def wo_mm(r, i, n):
        xs[r][i:i + PMO, n:n + PNO] += _dot(_ld(a_scr[r], i, i + PMO), _ld(wo_p, 0, D, slice(n, n + PNO)))

    def wo_steps(r, i0=0, i1=MB):
        return [P(wo_mm, r, i, n) for n in range(0, D, PNO) for i in range(i0, i1, PMO)]

    def ffn_up(c, r, i=0, pm=MB, n=0, pn=FC):
        g = _dot(_ld(xn[r], i, i + pm), w1_v[c, :, n:n + pn])
        u = _dot(_ld(xn[r], i, i + pm), w3_v[c, :, n:n + pn])
        _st(h_scr[r], i, g * jax.nn.sigmoid(g) * u, slice(n, n + pn))

    def up_steps(c, r, pm=MB, pn=FC, i0=0, i1=MB):
        return [P(ffn_up, c, r, i, pm, n, pn) for n in range(0, FC, pn) for i in range(i0, i1, pm)]

    def ffn_down(c, r, i, pm, n, pn):
        xs[r][i:i + pm, n:n + pn] += _dot(_ld(h_scr[r], i, i + pm), w2_v[c, :, n:n + pn])

    def down_steps(c, r, pm=MB, pn=NQ, i0=0, i1=MB):
        return [P(ffn_down, c, r, i, pm, n, pn) for n in range(0, D, pn) for i in range(i0, i1, pm)]

    mark('pro')
    flag[0] = 1
    queue = [cp_wq[0], cp_x0[0], cp_wq[1], cp_wq[2], cp_wq[3], cp_x0[1]] + cp_wk + [cp_wv]
    for c in queue[:INF]:
        c.start()
    queue = queue[INF:]

    def land(c):
        c.wait()
        if queue:
            queue.pop(0).start()

    k_scr[:, 0:HALO, :] = jnp.zeros((8, HALO, 128), F32)
    land(cp_wq[0])
    steps = permute_qkv_steps(0, [0])
    _merge(steps[:8])
    land(cp_x0[0])
    _merge(steps[8:], ln_steps(0, load_in=True, i0=0, i1=HB))
    mark(None)

    def q_slab(t, n):
        y = _dot(_ld(xn[0], 0, HB, slice(t * 256, (t + 1) * 256)),
                 _ld(wqkv_p[0], t * 256, (t + 1) * 256, slice(n, n + 256)))
        for j in range(n // 128, n // 128 + 2):
            yj = y[:, j * 128 - n:(j + 1) * 128 - n]
            if t:
                yj = q_scr[j, 0:HB, :] + yj
            q_scr[j, 0:HB, :] = yj * (DH ** -0.5 * LOG2E) if t == 3 else yj

    def phase(name):
        def deco(fn):
            mark(name)
            pl.when(flag[0] == 1)(fn)
            mark(None)
        return deco

    def layer(l):
        pend = []

        def run(name, main, *sides):
            pend.append((main, sides))
            if name in JOIN.split('.'):
                return
            work = list(pend)
            pend.clear()
            phase(name)(lambda: [_merge(m, *sd) for m, sd in work] and None)

        def halves(steps):
            return steps[:len(steps) // 2], steps[len(steps) // 2:]

        def first(steps, *waits):
            if l:
                return []
            for c in waits:
                c.wait()
            return steps

        def qkv(m, r):
            return proj_steps(m, [r], 0, D, *((PMP, PNP) if m == 0 or r == 0 else (PMV, PNV)))

        pwo = halves(permute_wo_steps())
        pb = va = vb = []
        for r in range(NB):
            if r == 0:
                if l:
                    run('Q0', qkv(0, r), ln_steps(NB - 1))
                    run('K0', qkv(1, r))
                else:
                    for t in range(4):
                        land(cp_wq[t + 1] if t < 3 else cp_x0[1])
                        run('Q0a', [P(q_slab, t, n) for n in range(0, D, 256)],
                            permute_qkv_steps(0, [t + 1]) if t < 3 else ln_steps(0, load_in=True, i0=HB))
                    for t in range(4):
                        land(cp_wk[t])
                        run('Q0b', [P(proj, 0, 0, i, 128, n, 128) for n in (256 * t, 256 * t + 128)
                                    for i in range(HB, MB, 128)], permute_qkv_steps(1, [t]))
                    for c in queue + [cp_x[1], cp_wo, cp_x[2], cp_x[3]]:
                        c.start()
                    k0 = halves(qkv(1, r))
                    run('K0a', k0[0])
                    run('K0b', k0[1], first(permute_qkv_steps(2), cp_wv))
                    for c in cp_ffn:
                        c.start()
            else:
                ln2 = ln_steps(r - 2) if r > 1 else []
                ln2 = {'Q': (ln2, [], []), 'K': ([], ln2, []), 'KV': ([],) + halves(ln2)}[LNP]
                run('Q%d' % r, qkv(0, r), pb, ln2[0], first(pwo[0], cp_wo) if r == 1 else [])
                run('K%d' % r, qkv(1, r), va, ln2[1], first(pwo[1]) if r == 1 else [])
            pa, pb = probs_steps(r, 0), probs_steps(r, 1)
            nxt = first(ln_steps(r + 1, load_in=True), cp_x[r + 1]) if r + 1 < NB else []
            if r == 0:
                run('V0', qkv(2, r), pa, nxt)
            else:
                run('V%d' % r, qkv(2, r), vb, nxt, ln2[2])
                run('O%d' % (r - 1), wo_steps(r - 1), pa)
            va, vb = halves(pv_steps(r))
        if l == 0:
            for c in cp_ffn:
                c.wait()

        def up(r):
            return up_steps(0, r, PM, PN)

        def down(r):
            return down_steps(0, r, PM, 256)

        run('F0a', up(0) + down(0), pb, ln_steps(NB - 2))
        run('F0b', up_steps(0, 1, PMV, PNV) + down_steps(0, 1, PMV, PND), va)
        run('F0c', up_steps(0, 2, PMV, PNV) + down_steps(0, 2, PMV, PND), vb)
        hb = MB // 2
        run('O3a', wo_steps(3, 0, hb))
        run('O3b', wo_steps(3, hb, MB), ln_steps(3, i0=0, i1=hb))
        run('F0d', up_steps(0, 3, PMD, PNDU, 0, hb), ln_steps(3, i0=hb))
        run('F0e', up_steps(0, 3, hb, FC, hb, MB) + down_steps(0, 3))

        mark('Floop')

        def chunk(c, carry):
            for r in range(NB):
                ffn_up(c, r)
            for r in range(NB):
                _merge(down_steps(c, r))
            return carry
        lax.fori_loop(1, NC - 1, chunk, 0)

        c = NC - 1
        for r in range(NB):
            if l == 0:
                if r:
                    run('L%d' % r, up_steps(c, r, PML, PNL) + down_steps(c, r, PML, 256), ln_steps(r - 1))
                else:
                    run('L0', up_steps(c, r) + down_steps(c, r))
            else:
                @phase('L%d' % r)
                def _():
                    _merge(up_steps(c, r))
                    ob = MB if r + 1 < NB else OB
                    for i in range(0, MB, ob):
                        _merge(down_steps(c, r, ob, NQ, i, i + ob))
                        io[r][i:i + ob, :] = xs[r][i:i + ob, :].astype(BF16)
                        cp_out(r, i, ob).start()

    for l in LAYERS:
        layer(l)
    for r in range(NB):
        cp_out(r, 0, MB).wait()


def _build(A_x, A_wqkv, A_wo, B_x, B_w1, B_w3, B_w2, R=8, RP=16, FC=256, NQ=256, NB=4, RL=32,
           JP=1, BAR='QKVO', PM=128, PN=128, PMV=128, PNV=128, PMP=128, PNP=128, PMO=128, PNO=128, PML=256, PNL=128, OB=128, LD=0, INF=4, PMD=256, PNDU=256, PND=128, JOIN='K1.K2.K3.O0.O1.O2.O3a.F0b.F0d.L0', LAYERS=(0, 1), DLY=4, LNP='KV', scopes=False):
    del B_x
    B, S, D = A_x.shape
    F = B_w1.shape[1]
    NC = F // FC
    MB = S // NB
    x = A_x.reshape(S, D)
    anyspec = pl.BlockSpec(memory_space=pl.ANY)
    out = pl.pallas_call(
        functools.partial(_kernel, R=R, RP=RP, FC=FC, NQ=NQ, RL=RL, JP=JP, BAR=BAR, scopes=scopes, PM=PM, PN=PN, PMV=PMV, PNV=PNV, PMP=PMP, PNP=PNP, PMO=PMO, PNO=PNO, PML=PML, PNL=PNL, OB=OB, LD=LD, INF=INF, PMD=PMD, PNDU=PNDU, PND=PND, JOIN=JOIN, LAYERS=LAYERS, DLY=DLY, LNP=LNP),
        in_specs=[anyspec] * 6,
        out_specs=anyspec,
        out_shape=jax.ShapeDtypeStruct((S, D), A_x.dtype),
        scratch_shapes=[
            pltpu.VMEM((3, D, D), BF16), [pltpu.VMEM((D // 2, D), U32)] * 3,
            pltpu.VMEM((D, D), BF16), pltpu.VMEM((D // 2, D), U32),
            pltpu.VMEM((NC, D, FC), BF16), pltpu.VMEM((NC, D, FC), BF16), pltpu.VMEM((NC, FC, D), BF16),
            [pltpu.VMEM((H * PAD, 128), U32)] * 2,
            pltpu.VMEM((8, S, 128), F32), pltpu.VMEM((8, S + HALO, 128), F32),
            [pltpu.VMEM((S + HALO, 128), F32)] * 8,
            [pltpu.VMEM((MB // 2, D), U32)] * NB,
            [pltpu.VMEM((MB, D), F32)] * NB, [pltpu.VMEM((MB // 2, D), U32)] * NB, [pltpu.VMEM((MB, D), BF16)] * NB,
            [pltpu.VMEM((MB // 2, FC), U32)] * NB,
            pltpu.SemaphoreType.DMA((NB,)), pltpu.SemaphoreType.DMA((13,)), pltpu.SemaphoreType.DMA((NB,)),
            pltpu.SMEM((1,), jnp.int32),
        ],
        compiler_params=pltpu.CompilerParams(vmem_limit_bytes=120 * 1024 * 1024),
    )(x, A_wqkv, A_wo, B_w1, B_w3, B_w2)
    return out.reshape(B, S, D)


@jax.jit
def pallas_interleave_layers__sliding_local_dilated__glu_gated_swiglu__prompt_kernel(
        A_x, A_wqkv, A_wo, B_x, B_w1, B_w3, B_w2):
    return _build(A_x, A_wqkv, A_wo, B_x, B_w1, B_w3, B_w2)
```

```python
import contextlib
import functools
import math
import jax
import jax.numpy as jnp
from jax import lax
import jax.experimental.pallas as pl
import jax.experimental.pallas.tpu as pltpu

H, DH, W, DIL = 32, 32, 8, 2
HALO = 16
PAD = DH + 1
SLOTS = (0, 1, 3, 2, 4, 5, 6)
EPS = 1e-5
LOG2E = math.log2(math.e)
F32, BF16, U32 = jnp.float32, jnp.bfloat16, jnp.uint32


def _ln(x):
    m = jnp.mean(x, axis=-1, keepdims=True)
    c = x - m
    v = jnp.mean(c * c, axis=-1, keepdims=True)
    return c * lax.rsqrt(v + EPS)


def _dot(a, b):
    return jnp.dot(a, b, preferred_element_type=F32)


def _ld(ref, r0, r1, cols=slice(None)):
    return pltpu.bitcast(ref[r0 // 2:r1 // 2, cols], BF16)


def _st(ref, r0, val, cols=slice(None)):
    ref[r0 // 2:(r0 + val.shape[0]) // 2, cols] = pltpu.bitcast(val.astype(BF16), U32)


def _lhs_operands(a11, a12, a21, a22):
    return (a11 + a22, a21 + a22, a11, a22, a11 + a12, a21 - a11, a12 - a22)


def _combine(m):
    m1, m2, m3, m4, m5, m6, m7 = m
    return m1 + m4 - m5 + m7, m3 + m5, m2 + m4, m1 - m2 + m3 + m6


def _merge(main, *sides):
    n = len(main)
    for i, f in enumerate(main):
        f()
        for s in sides:
            for g in s[len(s) * i // n:len(s) * (i + 1) // n]:
                g()


def _kernel(x_hbm, wqkv_hbm, wo_hbm, w1_hbm, w3_hbm, w2_hbm, o_hbm,
            wqkv_raw, wqkv_p, wo_raw, wo_p, wup, wdn, tr_scr, q_scr, k_scr,
            v_scr, a_scr, xs, xn, xa, io, ha, sem_x, sem_w, sem_f, sem_o, flag, *,
            R, RP, FC, RL, RL2, JP, PM, PN, PMV, PNV, PMP, PNP, PMO, PNO, OB, LD, INF, PMU, PNU, PMD, PND,
            PMF, PNF, PNG, JOIN, LAYERS, DLY, LNP, SUB, PREP, scopes):
    NB, MB, D = xs.shape
    HB, HD = MB // 2, D // 2
    S = NB * MB
    a_scr = [a_scr[r % 2] for r in range(NB)]
    NP = wdn.shape[0]
    P = functools.partial
    st = contextlib.ExitStack()

    def mark(name):
        st.close()
        if scopes and name:
            st.enter_context(jax.named_scope(name))

    cp_x = {r: pltpu.make_async_copy(x_hbm.at[r * MB:(r + 1) * MB, :], io[r], sem_x.at[r]) for r in range(1, NB)}

    def cp_out(r, i, n):
        return pltpu.make_async_copy(io[r].at[i:i + n, :], o_hbm.at[r * MB + i:r * MB + i + n, :], sem_o.at[r])

    cp_wq, cp_wk = [[pltpu.make_async_copy(wqkv_hbm.at[t * 256:(t + 1) * 256, m * D:(m + 1) * D],
                                           wqkv_raw.at[m, t * 256:(t + 1) * 256, :], sem_w.at[4 * m + t])
                     for t in range(4)] for m in range(2)]
    cp_wv = pltpu.make_async_copy(wqkv_hbm.at[:, 2 * D:3 * D], wqkv_raw.at[2], sem_w.at[8])
    cp_x0 = [pltpu.make_async_copy(x_hbm.at[i * HB:(i + 1) * HB, :], io[0].at[i * HB:(i + 1) * HB, :],
                                   sem_w.at[11 + i]) for i in range(2)]
    cp_wo = pltpu.make_async_copy(wo_hbm, wo_raw, sem_w.at[9])
    cp_ffn = []
    for p in range(NP):
        cps = [(w.at[:, c * FC:(c + 1) * FC], wup.at[c, s * HD:(s + 2) * HD, :])
               for c in (2 * p, 2 * p + 1) for w, s in ((w1_hbm, 1), (w3_hbm, 3))]
        cps += [(w2_hbm.at[2 * p * FC:(2 * p + 2) * FC, n:n + HD], wdn.at[p, s * FC:(s + 2) * FC, :])
                for n, s in ((0, 1), (HD, 3))]
        cp_ffn.append([pltpu.make_async_copy(a, b, sem_f.at[p]) for a, b in cps])

    def prep(w, c, rows, i, n):
        b11, b21, b12, b22 = [w[c, s * rows + i:s * rows + i + n, :].astype(F32) for s in (1, 2, 3, 4)]
        for s, val in ((0, b11 + b22), (2, b21 - b11), (3, b12 - b22), (5, b11 + b12), (6, b21 + b22)):
            w[c, s * rows + i:s * rows + i + n, :] = val.astype(BF16)

    def prep_steps(p):
        return [P(prep, w, c, rows, i, n)
                for w, c, rows, n in ((wup, 2 * p, HD, 32), (wup, 2 * p + 1, HD, 32), (wdn, p, FC, 16))
                for i in range(0, rows, n)]

    def stage(slot, i, val):
        for hh in range(4):
            h = 4 * i + hh
            tr_scr[slot][h * PAD:h * PAD + DH, :] = val[hh * DH:(hh + 1) * DH, :]

    def gather(slot, j):
        return jnp.concatenate([tr_scr[slot][pl.ds(4 * j + dd, H, stride=PAD), :] for dd in range(4)], axis=0)

    def qkv_in(m, t, i):
        blk = pltpu.bitcast(wqkv_raw[m, t * 256:(t + 1) * 256, i * 128:(i + 1) * 128], U32)
        stage(t % 2, i, blk.T)

    def qkv_out(m, t, j):
        wqkv_p[m][t * 128:(t + 1) * 128, j * 128:(j + 1) * 128] = gather(t % 2, j).T

    def permute_qkv_steps(m, ts=range(4)):
        return [P(f, m, t, i) for t in ts for f in (qkv_in, qkv_out) for i in range(8)]

    def wo_in(c, i):
        stage(c % 2, i, pltpu.bitcast(wo_raw[i * 128:(i + 1) * 128, c * 128:(c + 1) * 128].astype(F32), U32))

    def wo_out(c, j):
        _st(wo_p, j * 128, pltpu.bitcast(gather(c % 2, j), F32), slice(c * 128, (c + 1) * 128))

    def permute_wo_steps():
        return [P(f, c, i) for c in range(8) for f in (wo_in, wo_out) for i in range(8)]

    def proj(m, r, i, pm, n0, pn):
        y = _dot(_ld(xn[r], i, i + pm), _ld(wqkv_p[m], 0, D, slice(n0, n0 + pn)))
        if m == 0:
            y = y * (DH ** -0.5 * LOG2E)
        b = r * MB + i
        for j in range(n0 // 128, (n0 + pn) // 128):
            yj = y[:, j * 128 - n0:(j + 1) * 128 - n0]
            if m == 0:
                q_scr[j, b:b + pm, :] = yj
            elif m == 1:
                k_scr[j, HALO + b:HALO + b + pm, :] = yj
            else:
                v_scr[j][HALO + b:HALO + b + pm, :] = yj
                if b == 0:
                    v_scr[j][0:HALO, :] = jnp.broadcast_to(yj[0:1, :], (HALO, 128))

    def proj_steps(m, rs, n0=0, n1=D, pm=PM, pn=PN):
        return [P(proj, m, r, i, pm, n, pn) for n in range(n0, n1, pn) for r in rs for i in range(0, MB, pm)]

    def probs_steps(r, half):
        base = r * MB + half * (MB // 2)
        items = [(b, w) for b in range(base, base + MB // 2, R) for w in range(W)]
        s1, s2, done, qs = {}, {}, [], {}

        def step(t):
            if t < len(items):
                b, w = items[t]
                if w == 0:
                    qs[b] = [q_scr[j, b:b + R, :] for j in range(8)]
                p = None
                for j in range(8):
                    u = qs[b][j] * k_scr[j, HALO + b - DIL * w:HALO + b - DIL * w + R, :]
                    p = u if p is None else p + u
                s1[t] = (p, pltpu.roll(p, 64, 1))
            if 0 <= t - DLY < len(items):
                u, v = s1.pop(t - DLY)
                u = u + v
                s2[t - DLY] = (u, pltpu.roll(u, 32, 1))
            if t - 2 * DLY >= 0:
                b, w = items[t - 2 * DLY]
                u, v = s2.pop(t - 2 * DLY)
                p = u + v
                if b < DIL * w:
                    pos = b + lax.broadcasted_iota(jnp.int32, (R, 128), 0)
                    p = jnp.where(pos >= DIL * w, p, -1e9 * LOG2E)
                done.append(p)
                if w == W - 1:
                    mx = functools.reduce(jnp.maximum, done)
                    es = [jnp.exp2(p - mx) for p in done]
                    inv = 1.0 / functools.reduce(lambda u, v: u + v, es)
                    for w in range(W):
                        q_scr[w, b:b + R, :] = es[w] * inv
                    done.clear()
        return [P(step, t) for t in range(len(items) + 2 * DLY)]

    def pv(r, i, js):
        b = r * MB + i
        es = [q_scr[w, b:b + RP, :] for w in range(W)]
        for j in js:
            o = None
            for w in range(W):
                t = es[w] * v_scr[j][HALO + b - DIL * w:HALO + b - DIL * w + RP, :]
                o = t if o is None else o + t
            _st(a_scr[r], i, o, slice(j * 128, (j + 1) * 128))

    def pv_steps(r):
        return [P(pv, r, i, range(j, j + JP)) for i in range(0, MB, RP) for j in range(0, 8, JP)]

    def ln_steps(r, load_in=False, i0=0, i1=MB):
        rows = list(range(i0, i1, RL))
        mean, var = {}, {}

        def step(t):
            if t < len(rows):
                b = rows[t]
                if load_in:
                    x = io[r][b:b + RL, :].astype(F32)
                    xs[r, b:b + RL, :] = x
                else:
                    x = xs[r, b:b + RL, :]
                mean[b] = jnp.mean(x, axis=-1, keepdims=True)
            if 0 <= t - LD < len(rows):
                b = rows[t - LD]
                c = xs[r, b:b + RL, :] - mean[b]
                var[b] = jnp.mean(c * c, axis=-1, keepdims=True)
            if t - 2 * LD >= 0:
                b = rows[t - 2 * LD]
                c = xs[r, b:b + RL, :] - mean.pop(b)
                _st(xn[r], b, c * lax.rsqrt(var.pop(b) + EPS))
        return [P(step, t) for t in range(len(rows) + 2 * LD)]

    def wo_mm(r, i, n):
        xs[r, i:i + PMO, n:n + PNO] += _dot(_ld(a_scr[r], i, i + PMO), _ld(wo_p, 0, D, slice(n, n + PNO)))

    def wo_steps(r, i0=0, i1=MB):
        return [P(wo_mm, r, i, n) for n in range(0, D, PNO) for i in range(i0, i1, PMO)]

    def ln2_blk(r, b):
        top, bot = _ln(xs[r, b:b + RL2, :]), _ln(xs[r, HB + b:HB + b + RL2, :])
        for i, val in enumerate(_lhs_operands(top[:, :HD], top[:, HD:], bot[:, :HD], bot[:, HD:])):
            _st(xa.at[r, i], b, val)

    def ln2_steps(r):
        return [P(ln2_blk, r, b) for b in range(0, HB, RL2)]

    def ffn_up(p, r, slot, i, pm, n, pn):
        hs = []
        for c in (2 * p, 2 * p + 1):
            gt, ut, gb, ub = _combine([_dot(_ld(xa.at[r, t], i, i + pm), wup[c, s * HD:(s + 1) * HD, n:n + pn])
                                       for t, s in enumerate(SLOTS)])
            hs.append((gt * jax.nn.sigmoid(gt) * ut, gb * jax.nn.sigmoid(gb) * ub))
        for t, val in enumerate(_lhs_operands(hs[0][0], hs[1][0], hs[0][1], hs[1][1])):
            _st(ha.at[slot, t], i, val, slice(n, n + pn))

    def ffn_down(p, r, slot, i, pm, n, pn):
        c11, c12, c21, c22 = _combine([_dot(_ld(ha.at[slot, t], i, i + pm), wdn[p, s * FC:(s + 1) * FC, n:n + pn])
                                       for t, s in enumerate(SLOTS)])
        xs[r, i:i + pm, n:n + pn] += c11
        xs[r, i:i + pm, HD + n:HD + n + pn] += c12
        xs[r, HB + i:HB + i + pm, n:n + pn] += c21
        xs[r, HB + i:HB + i + pm, HD + n:HD + n + pn] += c22

    def up_steps(p, r, slot, pm=PMU, pn=PNU):
        return [P(ffn_up, p, r, slot, i, pm, n, pn) for n in range(0, FC, pn) for i in range(0, HB, pm)]

    def down_steps(p, r, slot, pm=PMD, pn=PND, i0=0, i1=HB):
        return [P(ffn_down, p, r, slot, i, pm, n, pn) for n in range(0, HD, pn) for i in range(i0, i1, pm)]

    def ffn_steps(p, r):
        return up_steps(p, r, r % 2) + down_steps(p, r, r % 2)

    mark('pro')
    flag[0] = 1
    queue = [cp_wq[0], cp_x0[0], cp_wq[1], cp_wq[2], cp_wq[3], cp_x0[1]] + cp_wk + [cp_wv]
    for c in queue[:INF]:
        c.start()
    queue = queue[INF:]

    def land(c):
        c.wait()
        if queue:
            queue.pop(0).start()

    k_scr[:, 0:HALO, :] = jnp.zeros((8, HALO, 128), F32)
    land(cp_wq[0])
    steps = permute_qkv_steps(0, [0])
    _merge(steps[:8])
    land(cp_x0[0])
    _merge(steps[8:], ln_steps(0, load_in=True, i0=0, i1=HB))
    mark(None)

    def q_slab(t, n):
        y = _dot(_ld(xn[0], 0, HB, slice(t * 256, (t + 1) * 256)),
                 _ld(wqkv_p[0], t * 256, (t + 1) * 256, slice(n, n + 256)))
        for j in range(n // 128, n // 128 + 2):
            yj = y[:, j * 128 - n:(j + 1) * 128 - n]
            if t:
                yj = q_scr[j, 0:HB, :] + yj
            q_scr[j, 0:HB, :] = yj * (DH ** -0.5 * LOG2E) if t == 3 else yj

    def phase(name):
        def deco(fn):
            mark(name)
            pl.when(flag[0] == 1)(fn)
            mark(None)
        return deco

    def layer(l):
        pend = []

        def run(name, main, *sides):
            n = SUB.count(name[0]) if name[1].isdigit() else 1
            if n > 1:
                for i in range(n):
                    cut = lambda s: s[len(s) * i // n:len(s) * (i + 1) // n]
                    phase(name)(lambda: _merge(cut(main), *map(cut, sides)))
                return
            pend.append((main, sides))
            if name in JOIN.split('.'):
                return
            work = list(pend)
            pend.clear()
            phase(name)(lambda: [_merge(m, *sd) for m, sd in work] and None)

        def halves(steps):
            return steps[:len(steps) // 2], steps[len(steps) // 2:]

        def first(steps, *waits):
            if l:
                return []
            for c in waits:
                c.wait()
            return steps

        def preps(name):
            ps = [p for p, nm in enumerate(PREP.split('.')) if nm == name]
            return first([s for p in ps for s in prep_steps(p)], *[c for p in ps for c in cp_ffn[p]])

        def qkv(m, r):
            return proj_steps(m, [r], 0, D, *((PMP, PNP) if m == 0 or r == 0 else (PMV, PNV)))

        pwo = halves(permute_wo_steps())
        pb = va = vb = []
        for r in range(NB):
            if r == 0:
                if l:
                    run('Q0', qkv(0, r), ln_steps(NB - 1))
                    run('K0', qkv(1, r))
                else:
                    for t in range(4):
                        land(cp_wq[t + 1] if t < 3 else cp_x0[1])
                        run('Q0a', [P(q_slab, t, n) for n in range(0, D, 256)],
                            permute_qkv_steps(0, [t + 1]) if t < 3 else ln_steps(0, load_in=True, i0=HB))
                    for t in range(4):
                        land(cp_wk[t])
                        run('Q0b', [P(proj, 0, 0, i, 128, n, 128) for n in (256 * t, 256 * t + 128)
                                    for i in range(HB, MB, 128)], permute_qkv_steps(1, [t]))
                    for c in queue + [cp_x[1], cp_wo, cp_x[2], cp_x[3]]:
                        c.start()
                    k0 = halves(qkv(1, r))
                    run('K0a', k0[0])
                    run('K0b', k0[1], first(permute_qkv_steps(2), cp_wv))
                    for cps in cp_ffn:
                        for c in cps:
                            c.start()
            else:
                ln2 = ln2_steps(r - 2) if r > 1 else []
                ln2 = {'Q': (ln2, [], []), 'K': ([], ln2, []), 'KV': ([],) + halves(ln2)}[LNP]
                run('Q%d' % r, qkv(0, r), pb, ln2[0], first(pwo[0], cp_wo) if r == 1 else [], preps('Q%d' % r))
                run('K%d' % r, qkv(1, r), va, ln2[1], preps('K%d' % r), first(pwo[1]) if r == 1 else [])
            pa, pb = probs_steps(r, 0), probs_steps(r, 1)
            nxt = first(ln_steps(r + 1, load_in=True), cp_x[r + 1]) if r + 1 < NB else []
            if r == 0:
                run('V0', qkv(2, r), pa, nxt)
            else:
                run('V%d' % r, qkv(2, r), vb, nxt, ln2[2], preps('V%d' % r))
                run('O%d' % (r - 1), wo_steps(r - 1), pa, preps('O%d' % (r - 1)))
            va, vb = halves(pv_steps(r))
        run('F0a', ffn_steps(0, 0), pb, ln2_steps(NB - 2))
        run('F0b', ffn_steps(0, 1), va + vb, preps('F0b'))
        run('O3', wo_steps(NB - 1), preps('O3'))
        run('F0c', ffn_steps(0, 2), ln2_steps(NB - 1))
        run('F0d', ffn_steps(0, 3), preps('F0d'))
        mark('Floop')

        def body(it, carry):
            p, half = 1 + it // 2, it % 2
            for u in range(2):
                _merge(up_steps(p, 2 * half + u, u, PMF, PNF))
            for u in range(2):
                _merge(down_steps(p, 2 * half + u, u, PMF, PNG))
            return carry
        lax.fori_loop(0, 2 * (NP - 2), body, 0)
        p = NP - 1
        for r in range(NB):
            if l == 0:
                run('L%d' % r, ffn_steps(p, r), ln_steps(r - 1) if r else [])
            else:
                @phase('L%d' % r)
                def _():
                    _merge(up_steps(p, r, r % 2))
                    ob = HB if r + 1 < NB else OB
                    for i in range(0, HB, ob):
                        _merge(down_steps(p, r, r % 2, min(ob, PMD), PND, i, i + ob))
                        for i0 in (i, HB + i):
                            io[r][i0:i0 + ob, :] = xs[r, i0:i0 + ob, :].astype(BF16)
                            cp_out(r, i0, ob).start()

    for l in LAYERS:
        layer(l)
    for r in range(NB):
        cp_out(r, 0, MB).wait()


def _build(A_x, A_wqkv, A_wo, B_x, B_w1, B_w3, B_w2, NB=4, **kw):
    cfg = dict(R=8, RP=16, FC=256, RL=32, RL2=16, JP=1, PM=128, PN=128, PMV=128, PNV=128, PMP=128, PNP=128,
               PMO=128, PNO=128, OB=128, LD=0, INF=4, PMU=256, PNU=256, PMD=256, PND=256, PMF=256, PNF=256, PNG=512,
               JOIN='K1.K2.K3.O0.O1.O2.O3.L0', LAYERS=(0, 1), DLY=6, LNP='KV', SUB='', PREP='K3.F0b.O3.F0d.K2.V2.V3', scopes=False)
    cfg.update(kw)
    FC = cfg['FC']
    del B_x
    B, S, D = A_x.shape
    F = B_w1.shape[1]
    NC = F // FC
    MB = S // NB
    x = A_x.reshape(S, D)
    anyspec = pl.BlockSpec(memory_space=pl.ANY)
    out = pl.pallas_call(
        functools.partial(_kernel, **cfg),
        in_specs=[anyspec] * 6,
        out_specs=anyspec,
        out_shape=jax.ShapeDtypeStruct((S, D), A_x.dtype),
        scratch_shapes=[
            pltpu.VMEM((3, D, D), BF16), [pltpu.VMEM((D // 2, D), U32)] * 3,
            pltpu.VMEM((D, D), BF16), pltpu.VMEM((D // 2, D), U32),
            pltpu.VMEM((NC, 7 * D // 2, FC), BF16), pltpu.VMEM((NC // 2, 7 * FC, D // 2), BF16),
            [pltpu.VMEM(((H + 1) * PAD + 7, 128), U32)] * 2,
            pltpu.VMEM((8, S, 128), F32), pltpu.VMEM((8, S + HALO, 128), F32),
            [pltpu.VMEM((S + HALO, 128), F32)] * 8,
            [pltpu.VMEM((MB // 2, D), U32)] * 2,
            pltpu.VMEM((NB, MB, D), F32), [pltpu.VMEM((MB // 2, D), U32)] * NB,
            pltpu.VMEM((NB, 7, MB // 4, D // 2), U32), [pltpu.VMEM((MB, D), BF16)] * NB,
            pltpu.VMEM((2, 7, MB // 4, FC), U32),
            pltpu.SemaphoreType.DMA((NB,)), pltpu.SemaphoreType.DMA((13,)), pltpu.SemaphoreType.DMA((NC // 2,)), pltpu.SemaphoreType.DMA((NB,)),
            pltpu.SMEM((1,), jnp.int32),
        ],
        compiler_params=pltpu.CompilerParams(vmem_limit_bytes=126 * 1024 * 1024),
    )(x, A_wqkv, A_wo, B_w1, B_w3, B_w2)
    return out.reshape(B, S, D)


@jax.jit
def pallas_interleave_layers__sliding_local_dilated__glu_gated_swiglu__prompt_kernel(
        A_x, A_wqkv, A_wo, B_x, B_w1, B_w3, B_w2):
    return _build(A_x, A_wqkv, A_wo, B_x, B_w1, B_w3, B_w2)
```

```python
import contextlib
import functools
import math
import jax
import jax.numpy as jnp
from jax import lax
import jax.experimental.pallas as pl
import jax.experimental.pallas.tpu as pltpu

H, DH, W, DIL = 32, 32, 8, 2
HALO = 16
PAD = DH + 1
SLOTS = (0, 1, 3, 2, 4, 5, 6)
EPS = 1e-5
LOG2E = math.log2(math.e)
F32, BF16, U32 = jnp.float32, jnp.bfloat16, jnp.uint32


def _ln(x):
    m = jnp.mean(x, axis=-1, keepdims=True)
    c = x - m
    v = jnp.mean(c * c, axis=-1, keepdims=True)
    return c * lax.rsqrt(v + EPS)


def _dot(a, b):
    return jnp.dot(a, b, preferred_element_type=F32)


def _ld(ref, r0, r1, cols=slice(None)):
    return pltpu.bitcast(ref[r0 // 2:r1 // 2, cols], BF16)


def _st(ref, r0, val, cols=slice(None)):
    ref[r0 // 2:(r0 + val.shape[0]) // 2, cols] = pltpu.bitcast(val.astype(BF16), U32)


def _lhs_operands(a11, a12, a21, a22):
    return (a11 + a22, a21 + a22, a11, a22, a11 + a12, a21 - a11, a12 - a22)


def _rhs_operands(b11, b12, b21, b22):
    return ((0, b11 + b22), (2, b21 - b11), (3, b12 - b22), (5, b11 + b12), (6, b21 + b22))


def _combine(m):
    m1, m2, m3, m4, m5, m6, m7 = m
    return m1 + m4 - m5 + m7, m3 + m5, m2 + m4, m1 - m2 + m3 + m6


def _merge(main, *sides):
    n = len(main)
    for i, f in enumerate(main):
        f()
        for s in sides:
            for g in s[len(s) * i // n:len(s) * (i + 1) // n]:
                g()


def _kernel(x_hbm, wqkv_hbm, wo_hbm, w1_hbm, w3_hbm, w2_hbm, o_hbm,
            wqkv_raw, wqkv_p, wo_raw, wo_p, wup, wdn, tr_scr, q_scr, k_scr,
            v_scr, a_scr, xs, xn0, xa, io, ha, sem_x, sem_w, sem_f, sem_o, flag, *,
            R, RP, FC, RL, PMP, PNP, PMO, PNO, OB, INF, PMU, PNU, PMD, PND,
            PMF, PNF, PNG, JOIN, LAYERS, DLY, LNP, SUB, PREP, scopes):
    NB, MB, D = xs.shape
    HB, HD = MB // 2, D // 2
    S = NB * MB
    a_scr = [a_scr[r % 2] for r in range(NB)]
    NP = wdn.shape[0]
    P = functools.partial
    st = contextlib.ExitStack()

    def mark(name):
        st.close()
        if scopes and name:
            st.enter_context(jax.named_scope(name))

    cp_x = {r: pltpu.make_async_copy(x_hbm.at[r * MB:(r + 1) * MB, :], io[r], sem_x.at[r]) for r in range(1, NB)}

    def cp_out(r, i, n):
        return pltpu.make_async_copy(io[r].at[i:i + n, :], o_hbm.at[r * MB + i:r * MB + i + n, :], sem_o.at[r])

    cp_wq, cp_wk = [[pltpu.make_async_copy(wqkv_hbm.at[t * 256:(t + 1) * 256, m * D:(m + 1) * D],
                                           wqkv_raw.at[m, t * 256:(t + 1) * 256, :], sem_w.at[4 * m + t])
                     for t in range(4)] for m in range(2)]
    cp_wv = pltpu.make_async_copy(wqkv_hbm.at[:, 2 * D:3 * D], wqkv_raw.at[2], sem_w.at[8])
    cp_x0 = [pltpu.make_async_copy(x_hbm.at[i * HB:(i + 1) * HB, :], io[0].at[i * HB:(i + 1) * HB, :],
                                   sem_w.at[11 + i]) for i in range(2)]
    cp_wo = pltpu.make_async_copy(wo_hbm, wo_raw, sem_w.at[9])
    cp_ffn = []
    for p in range(NP):
        cps = [(w.at[:, c * FC:(c + 1) * FC], wup.at[c, s * HD:(s + 2) * HD, :])
               for c in (2 * p, 2 * p + 1) for w, s in ((w1_hbm, 1), (w3_hbm, 3))]
        cps += [(w2_hbm.at[2 * p * FC:(2 * p + 2) * FC, n:n + HD], wdn.at[p, s * FC:(s + 2) * FC, :])
                for n, s in ((0, 1), (HD, 3))]
        cp_ffn.append([pltpu.make_async_copy(a, b, sem_f.at[p]) for a, b in cps])

    def prep(w, c, rows, i, n):
        b11, b21, b12, b22 = [w[c, s * rows + i:s * rows + i + n, :].astype(F32) for s in (1, 2, 3, 4)]
        for s, val in _rhs_operands(b11, b12, b21, b22):
            w[c, s * rows + i:s * rows + i + n, :] = val.astype(BF16)

    def prep_steps(p):
        return [P(prep, w, c, rows, i, n)
                for w, c, rows, n in ((wup, 2 * p, HD, 32), (wup, 2 * p + 1, HD, 32), (wdn, p, FC, 16))
                for i in range(0, rows, n)]

    def stage(slot, i, val):
        for hh in range(4):
            h = 4 * i + hh
            tr_scr[slot][h * PAD:h * PAD + DH, :] = val[hh * DH:(hh + 1) * DH, :]

    def gather(slot, j):
        return jnp.concatenate([tr_scr[slot][pl.ds(4 * j + dd, H, stride=PAD), :] for dd in range(4)], axis=0)

    def qkv_in(m, t, i):
        blk = pltpu.bitcast(wqkv_raw[m, t * 256:(t + 1) * 256, i * 128:(i + 1) * 128], U32)
        stage(t % 2, i, blk.T)

    def qkv_out(m, t, j):
        row = (1 + t // 2 + 2 * (j // 4)) * (HD // 2) + (t % 2) * 128
        wqkv_p[m][row:row + 128, (j % 4) * 128:(j % 4 + 1) * 128] = gather(t % 2, j).T

    def permute_qkv_steps(m, ts=range(4)):
        return [P(f, m, t, i) for t in ts for f in (qkv_in, qkv_out) for i in range(8)]

    def wo_in(c, i):
        stage(c % 2, i, pltpu.bitcast(wo_raw[i * 128:(i + 1) * 128, c * 128:(c + 1) * 128].astype(F32), U32))

    def wo_out(c, j):
        _st(wo_p, (1 + 2 * (c // 4)) * HD + j * 128, pltpu.bitcast(gather(c % 2, j), F32),
            slice((c % 4) * 128, (c % 4 + 1) * 128))

    def permute_wo_steps():
        return [P(f, c, i) for c in range(8) for f in (wo_in, wo_out) for i in range(8)]

    def prep_proj(w, i):
        b11, b21, b12, b22 = [_ld(w, s * HD + i, s * HD + i + 16).astype(F32) for s in (1, 2, 3, 4)]
        for s, val in _rhs_operands(b11, b12, b21, b22):
            _st(w, s * HD + i, val)

    def prep_proj_steps(w):
        return [P(prep_proj, w, i) for i in range(0, HD, 16)]

    def strassen_steps(lhs, w, pm, pn, emit):
        def product(ms, t, i, n):
            s = SLOTS[t]
            ms.append(_dot(_ld(lhs.at[t], i, i + pm), _ld(w, s * HD, (s + 1) * HD, slice(n, n + pn))))
            if t == 6:
                emit(i, n, *_combine(ms))
        steps = []
        for n in range(0, HD, pn):
            for i in range(0, HB, pm):
                ms = []
                steps += [P(product, ms, t, i, n) for t in range(7)]
        return steps

    def put_qkv(m, b, n, y):
        if m == 0:
            y = y * (DH ** -0.5 * LOG2E)
        rows = y.shape[0]
        for j in range(n // 128, (n + y.shape[1]) // 128):
            yj = y[:, j * 128 - n:(j + 1) * 128 - n]
            if m == 0:
                q_scr[j, b:b + rows, :] = yj
            elif m == 1:
                k_scr[j, HALO + b:HALO + b + rows, :] = yj
            else:
                v_scr[j][HALO + b:HALO + b + rows, :] = yj
                if b == 0:
                    v_scr[j][0:HALO, :] = jnp.broadcast_to(yj[0:1, :], (HALO, 128))

    def qkv(m, r):
        def emit(i, n, c11, c12, c21, c22):
            for di, dn, y in ((0, 0, c11), (0, HD, c12), (HB, 0, c21), (HB, HD, c22)):
                put_qkv(m, r * MB + i + di, n + dn, y)
        return strassen_steps(xa.at[r], wqkv_p[m], PMP, PNP, emit)

    def w_plain(m, k0, k1, n, pn):
        row = (1 + 2 * (n // HD)) * HD
        return _ld(wqkv_p[m], row + k0, row + k1, slice(n % HD, n % HD + pn))

    def proj_plain(m, i, n):
        put_qkv(m, i, n, _dot(_ld(xn0, i, i + 128), w_plain(m, 0, D, n, 128)))

    def probs_steps(r, half):
        base = r * MB + half * (MB // 2)
        items = [(b, w) for b in range(base, base + MB // 2, R) for w in range(W)]
        s1, s2, done, qs = {}, {}, [], {}

        def step(t):
            if t < len(items):
                b, w = items[t]
                if w == 0:
                    qs[b] = [q_scr[j, b:b + R, :] for j in range(8)]
                p = None
                for j in range(8):
                    u = qs[b][j] * k_scr[j, HALO + b - DIL * w:HALO + b - DIL * w + R, :]
                    p = u if p is None else p + u
                s1[t] = (p, pltpu.roll(p, 64, 1))
            if 0 <= t - DLY < len(items):
                u, v = s1.pop(t - DLY)
                u = u + v
                s2[t - DLY] = (u, pltpu.roll(u, 32, 1))
            if t - 2 * DLY >= 0:
                b, w = items[t - 2 * DLY]
                u, v = s2.pop(t - 2 * DLY)
                p = u + v
                if b < DIL * w:
                    pos = b + lax.broadcasted_iota(jnp.int32, (R, 128), 0)
                    p = jnp.where(pos >= DIL * w, p, -1e9 * LOG2E)
                done.append(p)
                if w == W - 1:
                    mx = functools.reduce(jnp.maximum, done)
                    es = [jnp.exp2(p - mx) for p in done]
                    inv = 1.0 / functools.reduce(lambda u, v: u + v, es)
                    for w in range(W):
                        q_scr[w, b:b + R, :] = es[w] * inv
                    done.clear()
        return [P(step, t) for t in range(len(items) + 2 * DLY)]

    def pv(b, j):
        o = None
        for w in range(W):
            t = q_scr[w, b:b + RP, :] * v_scr[j][HALO + b - DIL * w:HALO + b - DIL * w + RP, :]
            o = t if o is None else o + t
        return o

    def pv_steps(r):
        def step(os, i, j, di, dj):
            os.append(pv(r * MB + i + di, j + dj))
            if len(os) == 4:
                for t, val in enumerate(_lhs_operands(*os)):
                    _st(a_scr[r].at[t], i, val, slice(j * 128, (j + 1) * 128))
        steps = []
        for i in range(0, HB, RP):
            for j in range(4):
                os = []
                steps += [P(step, os, i, j, di, dj) for di in (0, HB) for dj in (0, 4)]
        return steps

    def load_x(r, b):
        x = io[r][b:b + RL, :].astype(F32)
        xs[r, b:b + RL, :] = x
        return x

    def ln_blk(r, b, from_input):
        top, bot = [_ln(load_x(r, i) if from_input else xs[r, i:i + RL, :]) for i in (b, HB + b)]
        for t, val in enumerate(_lhs_operands(top[:, :HD], top[:, HD:], bot[:, :HD], bot[:, HD:])):
            _st(xa.at[r, t], b, val)

    def ln_steps(r, from_input=False):
        return [P(ln_blk, r, b, from_input) for b in range(0, HB, RL)]

    def ln_plain_steps(i0, i1):
        def step(b):
            _st(xn0, b, _ln(load_x(0, b)))
        return [P(step, b) for b in range(i0, i1, RL)]

    def wo_steps(r):
        def emit(i, n, c11, c12, c21, c22):
            for di, dn, y in ((0, 0, c11), (0, HD, c12), (HB, 0, c21), (HB, HD, c22)):
                xs[r, i + di:i + di + PMO, n + dn:n + dn + PNO] += y
        return strassen_steps(a_scr[r], wo_p, PMO, PNO, emit)

    def ffn_up(p, r, slot, i, pm, n, pn):
        hs = []
        for c in (2 * p, 2 * p + 1):
            gt, ut, gb, ub = _combine([_dot(_ld(xa.at[r, t], i, i + pm), wup[c, s * HD:(s + 1) * HD, n:n + pn])
                                       for t, s in enumerate(SLOTS)])
            hs.append((gt * jax.nn.sigmoid(gt) * ut, gb * jax.nn.sigmoid(gb) * ub))
        for t, val in enumerate(_lhs_operands(hs[0][0], hs[1][0], hs[0][1], hs[1][1])):
            _st(ha.at[slot, t], i, val, slice(n, n + pn))

    def ffn_down(p, r, slot, i, pm, n, pn):
        c11, c12, c21, c22 = _combine([_dot(_ld(ha.at[slot, t], i, i + pm), wdn[p, s * FC:(s + 1) * FC, n:n + pn])
                                       for t, s in enumerate(SLOTS)])
        xs[r, i:i + pm, n:n + pn] += c11
        xs[r, i:i + pm, HD + n:HD + n + pn] += c12
        xs[r, HB + i:HB + i + pm, n:n + pn] += c21
        xs[r, HB + i:HB + i + pm, HD + n:HD + n + pn] += c22

    def up_steps(p, r, slot, pm=PMU, pn=PNU):
        return [P(ffn_up, p, r, slot, i, pm, n, pn) for n in range(0, FC, pn) for i in range(0, HB, pm)]

    def down_steps(p, r, slot, pm=PMD, pn=PND, i0=0, i1=HB):
        return [P(ffn_down, p, r, slot, i, pm, n, pn) for n in range(0, HD, pn) for i in range(i0, i1, pm)]

    def ffn_steps(p, r):
        return up_steps(p, r, r % 2) + down_steps(p, r, r % 2)

    mark('pro')
    flag[0] = 1
    queue = [cp_wq[0], cp_x0[0], cp_wq[1], cp_wq[2], cp_wq[3], cp_x0[1]] + cp_wk + [cp_wv]
    for c in queue[:INF]:
        c.start()
    queue = queue[INF:]

    def land(c):
        c.wait()
        if queue:
            queue.pop(0).start()

    k_scr[:, 0:HALO, :] = jnp.zeros((8, HALO, 128), F32)
    land(cp_wq[0])
    steps = permute_qkv_steps(0, [0])
    _merge(steps[:8])
    land(cp_x0[0])
    _merge(steps[8:], ln_plain_steps(0, HB))
    mark(None)

    def q_slab(t, n):
        y = _dot(_ld(xn0, 0, HB, slice(t * 256, (t + 1) * 256)), w_plain(0, t * 256, (t + 1) * 256, n, 256))
        for j in range(n // 128, n // 128 + 2):
            yj = y[:, j * 128 - n:(j + 1) * 128 - n]
            if t:
                yj = q_scr[j, 0:HB, :] + yj
            q_scr[j, 0:HB, :] = yj * (DH ** -0.5 * LOG2E) if t == 3 else yj

    def phase(name):
        def deco(fn):
            mark(name)
            pl.when(flag[0] == 1)(fn)
            mark(None)
        return deco

    def layer(l):
        pend = []

        def run(name, main, *sides):
            n = SUB.count(name[0]) if name[1].isdigit() else 1
            if n > 1:
                for i in range(n):
                    cut = lambda s: s[len(s) * i // n:len(s) * (i + 1) // n]
                    phase(name)(lambda: _merge(cut(main), *map(cut, sides)))
                return
            pend.append((main, sides))
            if name in JOIN.split('.'):
                return
            work = list(pend)
            pend.clear()
            phase(name)(lambda: [_merge(m, *sd) for m, sd in work] and None)

        def halves(steps):
            return steps[:len(steps) // 2], steps[len(steps) // 2:]

        def first(steps, *waits):
            if l:
                return []
            for c in waits:
                c.wait()
            return steps

        def preps(name):
            ps = [p for p, nm in enumerate(PREP.split('.')) if nm == name]
            return first([s for p in ps for s in prep_steps(p)], *[c for p in ps for c in cp_ffn[p]])

        pwo = halves(permute_wo_steps())
        pb = va = vb = []
        for r in range(NB):
            if r == 0:
                if l:
                    run('Q0', qkv(0, r), ln_steps(NB - 1))
                    run('K0', qkv(1, r))
                else:
                    for t in range(4):
                        land(cp_wq[t + 1] if t < 3 else cp_x0[1])
                        run('Q0a', [P(q_slab, t, n) for n in range(0, D, 256)],
                            permute_qkv_steps(0, [t + 1]) if t < 3 else ln_plain_steps(HB, MB))
                    for t in range(4):
                        land(cp_wk[t])
                        run('Q0b', [P(proj_plain, 0, i, n) for n in (256 * t, 256 * t + 128)
                                    for i in range(HB, MB, 128)], permute_qkv_steps(1, [t]))
                    for c in queue + [cp_x[1], cp_wo, cp_x[2], cp_x[3]]:
                        c.start()
                    k0 = halves([P(proj_plain, 1, i, n) for n in range(0, D, 128) for i in range(0, MB, 128)])
                    run('K0a', k0[0], prep_proj_steps(wqkv_p[0]), ln_steps(0))
                    run('K0b', k0[1], first(permute_qkv_steps(2) + prep_proj_steps(wqkv_p[2]), cp_wv))
                    for cps in cp_ffn:
                        for c in cps:
                            c.start()
            else:
                ln2 = ln_steps(r - 2) if r > 1 else []
                ln2 = {'Q': (ln2, [], []), 'K': ([], ln2, []), 'KV': ([],) + halves(ln2)}[LNP]
                run('Q%d' % r, qkv(0, r), pb, ln2[0], first(pwo[0] + prep_proj_steps(wqkv_p[1]), cp_wo) if r == 1 else [], preps('Q%d' % r))
                run('K%d' % r, qkv(1, r), va, ln2[1], preps('K%d' % r), first(pwo[1]) if r == 1 else [])
            pa, pb = probs_steps(r, 0), probs_steps(r, 1)
            nxt = first(ln_steps(r + 1, True), cp_x[r + 1]) if r + 1 < NB else []
            if r == 0:
                run('V0', qkv(2, r), pa, nxt)
            else:
                run('V%d' % r, qkv(2, r), vb, nxt, ln2[2], preps('V%d' % r),
                    first(prep_proj_steps(wo_p)) if r == 1 else [])
                run('O%d' % (r - 1), wo_steps(r - 1), pa, preps('O%d' % (r - 1)))
            va, vb = halves(pv_steps(r))
        run('F0a', ffn_steps(0, 0), pb, ln_steps(NB - 2))
        run('F0b', ffn_steps(0, 1), va + vb, preps('F0b'))
        run('O3', wo_steps(NB - 1), preps('O3'))
        run('F0c', ffn_steps(0, 2), ln_steps(NB - 1))
        run('F0d', ffn_steps(0, 3), preps('F0d'))
        mark('Floop')

        def body(it, carry):
            p, half = 1 + it // 2, it % 2
            for u in range(2):
                _merge(up_steps(p, 2 * half + u, u, PMF, PNF))
            for u in range(2):
                _merge(down_steps(p, 2 * half + u, u, PMF, PNG))
            return carry
        lax.fori_loop(0, 2 * (NP - 2), body, 0)
        p = NP - 1
        for r in range(NB):
            if l == 0:
                run('L%d' % r, ffn_steps(p, r), ln_steps(r - 1) if r else [])
            else:
                @phase('L%d' % r)
                def _():
                    _merge(up_steps(p, r, r % 2))
                    ob = HB if r + 1 < NB else OB
                    for i in range(0, HB, ob):
                        _merge(down_steps(p, r, r % 2, min(ob, PMD), PND, i, i + ob))
                        for i0 in (i, HB + i):
                            io[r][i0:i0 + ob, :] = xs[r, i0:i0 + ob, :].astype(BF16)
                            cp_out(r, i0, ob).start()

    for l in LAYERS:
        layer(l)
    for r in range(NB):
        cp_out(r, 0, MB).wait()


def _build(A_x, A_wqkv, A_wo, B_x, B_w1, B_w3, B_w2, NB=4, **kw):
    cfg = dict(R=8, RP=16, FC=256, RL=16, PMP=128, PNP=128,
               PMO=128, PNO=128, OB=128, INF=4, PMU=256, PNU=256, PMD=256, PND=256, PMF=256, PNF=256, PNG=512,
               JOIN='K1.K2.K3.O0.O1.O2.O3.L0', LAYERS=(0, 1), DLY=6, LNP='KV', SUB='', PREP='K3.F0b.O3.F0d.K2.V2.V3', scopes=False)
    cfg.update(kw)
    FC = cfg['FC']
    del B_x
    B, S, D = A_x.shape
    F = B_w1.shape[1]
    NC = F // FC
    MB = S // NB
    x = A_x.reshape(S, D)
    anyspec = pl.BlockSpec(memory_space=pl.ANY)
    out = pl.pallas_call(
        functools.partial(_kernel, **cfg),
        in_specs=[anyspec] * 6,
        out_specs=anyspec,
        out_shape=jax.ShapeDtypeStruct((S, D), A_x.dtype),
        scratch_shapes=[
            pltpu.VMEM((3, D, D), BF16), [pltpu.VMEM((7 * D // 4, D // 2), U32)] * 3,
            pltpu.VMEM((D, D), BF16), pltpu.VMEM((7 * D // 4, D // 2), U32),
            pltpu.VMEM((NC, 7 * D // 2, FC), BF16), pltpu.VMEM((NC // 2, 7 * FC, D // 2), BF16),
            [pltpu.VMEM(((H + 1) * PAD + 7, 128), U32)] * 2,
            pltpu.VMEM((8, S, 128), F32), pltpu.VMEM((8, S + HALO, 128), F32),
            [pltpu.VMEM((S + HALO, 128), F32)] * 8,
            [pltpu.VMEM((7, MB // 4, D // 2), U32)] * 2,
            pltpu.VMEM((NB, MB, D), F32), pltpu.VMEM((MB // 2, D), U32),
            pltpu.VMEM((NB, 7, MB // 4, D // 2), U32), [pltpu.VMEM((MB, D), BF16)] * NB,
            pltpu.VMEM((2, 7, MB // 4, FC), U32),
            pltpu.SemaphoreType.DMA((NB,)), pltpu.SemaphoreType.DMA((13,)), pltpu.SemaphoreType.DMA((NC // 2,)), pltpu.SemaphoreType.DMA((NB,)),
            pltpu.SMEM((1,), jnp.int32),
        ],
        compiler_params=pltpu.CompilerParams(vmem_limit_bytes=126 * 1024 * 1024),
    )(x, A_wqkv, A_wo, B_w1, B_w3, B_w2)
    return out.reshape(B, S, D)


@jax.jit
def pallas_interleave_layers__sliding_local_dilated__glu_gated_swiglu__prompt_kernel(
        A_x, A_wqkv, A_wo, B_x, B_w1, B_w3, B_w2):
    return _build(A_x, A_wqkv, A_wo, B_x, B_w1, B_w3, B_w2)
```

```python
import functools
import math
import jax
import jax.numpy as jnp
from jax import lax
import jax.experimental.pallas as pl
import jax.experimental.pallas.tpu as pltpu

H, DH, W, DIL = 32, 32, 8, 2
EPS = 1e-5
NB = 4
FC = 256
HALO = 16
PAD = DH + 1
R, RP, RL = 8, 16, 32
DLY = 4
SLOTS = (0, 1, 3, 2, 4, 5, 6)
LOG2E = math.log2(math.e)
QSCALE = DH ** -0.5 * LOG2E
F32, BF16, U32 = jnp.float32, jnp.bfloat16, jnp.uint32


def _ln(x):
    m = jnp.mean(x, axis=-1, keepdims=True)
    c = x - m
    v = jnp.mean(c * c, axis=-1, keepdims=True)
    return c * lax.rsqrt(v + EPS)


def _silu(g):
    hg = 0.5 * g
    return hg * jnp.tanh(hg) + hg


def _dot(a, b):
    return jnp.dot(a, b, preferred_element_type=F32)


def _ld(ref, r0, r1, cols=slice(None)):
    return pltpu.bitcast(ref[r0 // 2:r1 // 2, cols], BF16)


def _st(ref, r0, val, cols=slice(None)):
    ref[r0 // 2:(r0 + val.shape[0]) // 2, cols] = pltpu.bitcast(val.astype(BF16), U32)


def _lhs_operands(a11, a12, a21, a22):
    return (a11 + a22, a21 + a22, a11, a22, a11 + a12, a21 - a11, a12 - a22)


def _rhs_operands(b11, b12, b21, b22):
    return ((0, b11 + b22), (2, b21 - b11), (3, b12 - b22), (5, b11 + b12), (6, b21 + b22))


def _combine(m):
    m1, m2, m3, m4, m5, m6, m7 = m
    return m1 + m4 - m5 + m7, m3 + m5, m2 + m4, m1 - m2 + m3 + m6


def _zip(main, side):
    n, out = len(main), []
    for i, f in enumerate(main):
        out += [f] + side[len(side) * i // n:len(side) * (i + 1) // n]
    return out


def _merge(main, *sides):
    n = len(main)
    for i, f in enumerate(main):
        f()
        for s in sides:
            for g in s[len(s) * i // n:len(s) * (i + 1) // n]:
                g()


def _kernel(x_hbm, wqkv_hbm, wo_hbm, w1_hbm, w3_hbm, w2_hbm, o_hbm,
            wqkv_raw, wqkv_p, wo_raw, wo_p, wup, wdn, tr_scr, q_scr, k_scr,
            v_scr, a_scr, xs, xn0, xa, io, ha, sem_x, sem_w, sem_f, sem_o, flag):
    _, MB, D = xs.shape
    HB, HD = MB // 2, D // 2
    a_scr = [a_scr[r % 2] for r in range(NB)]
    NP = wdn.shape[0]
    P = functools.partial

    cp_x = {r: pltpu.make_async_copy(x_hbm.at[r * MB:(r + 1) * MB, :], io[r], sem_x.at[r]) for r in range(1, NB)}

    def cp_out(r, i, n):
        return pltpu.make_async_copy(io[r].at[i:i + n, :], o_hbm.at[r * MB + i:r * MB + i + n, :], sem_o.at[r])

    cp_wq, cp_wk = [[pltpu.make_async_copy(wqkv_hbm.at[t * 256:(t + 1) * 256, m * D:(m + 1) * D],
                                           wqkv_raw.at[m, t * 256:(t + 1) * 256, :], sem_w.at[4 * m + t])
                     for t in range(4)] for m in range(2)]
    cp_wv = pltpu.make_async_copy(wqkv_hbm.at[:, 2 * D:3 * D], wqkv_raw.at[2], sem_w.at[8])
    cp_x0 = [pltpu.make_async_copy(x_hbm.at[i * HB:(i + 1) * HB, :], io[0].at[i * HB:(i + 1) * HB, :],
                                   sem_w.at[11 + i]) for i in range(2)]
    cp_wo = pltpu.make_async_copy(wo_hbm, wo_raw, sem_w.at[9])
    cp_ffn = []
    for p in range(NP):
        cps = [(w.at[:, c * FC:(c + 1) * FC], wup.at[c, s * HD:(s + 2) * HD, :])
               for c in (2 * p, 2 * p + 1) for w, s in ((w1_hbm, 1), (w3_hbm, 3))]
        cps += [(w2_hbm.at[2 * p * FC:(2 * p + 2) * FC, n:n + HD], wdn.at[p, s * FC:(s + 2) * FC, :])
                for n, s in ((0, 1), (HD, 3))]
        cp_ffn.append([pltpu.make_async_copy(a, b, sem_f.at[p]) for a, b in cps])

    def prep(w, c, rows, i, n):
        b11, b21, b12, b22 = [w[c, s * rows + i:s * rows + i + n, :].astype(F32) for s in (1, 2, 3, 4)]
        for s, val in _rhs_operands(b11, b12, b21, b22):
            w[c, s * rows + i:s * rows + i + n, :] = val.astype(BF16)

    def prep_steps(p):
        return [P(prep, w, c, rows, i, n)
                for w, c, rows, n in ((wup, 2 * p, HD, 32), (wup, 2 * p + 1, HD, 32), (wdn, p, FC, 16))
                for i in range(0, rows, n)]

    def stage(slot, i, val):
        for hh in range(4):
            h = 4 * i + hh
            tr_scr[slot][h * PAD:h * PAD + DH, :] = val[hh * DH:(hh + 1) * DH, :]

    def gather(slot, j):
        return jnp.concatenate([tr_scr[slot][pl.ds(4 * j + dd, H, stride=PAD), :] for dd in range(4)], axis=0)

    def qkv_in(m, t, i):
        blk = pltpu.bitcast(wqkv_raw[m, t * 256:(t + 1) * 256, i * 128:(i + 1) * 128], U32)
        stage(t % 2, i, blk.T)

    def qkv_out(m, t, j):
        row = (1 + t // 2 + 2 * (j // 4)) * (HD // 2) + (t % 2) * 128
        wqkv_p[m][row:row + 128, (j % 4) * 128:(j % 4 + 1) * 128] = gather(t % 2, j).T

    def permute_qkv_steps(m, ts=range(4)):
        return [P(f, m, t, i) for t in ts for f in (qkv_in, qkv_out) for i in range(8)]

    def wo_in(c, i):
        stage(c % 2, i, pltpu.bitcast(wo_raw[i * 128:(i + 1) * 128, c * 128:(c + 1) * 128].astype(F32), U32))

    def wo_out(c, j):
        _st(wo_p, (1 + 2 * (c // 4)) * HD + j * 128, pltpu.bitcast(gather(c % 2, j), F32),
            slice((c % 4) * 128, (c % 4 + 1) * 128))

    def permute_wo_steps():
        return [P(f, c, i) for c in range(8) for f in (wo_in, wo_out) for i in range(8)]

    def prep_proj(w, i):
        b11, b21, b12, b22 = [_ld(w, s * HD + i, s * HD + i + 16).astype(F32) for s in (1, 2, 3, 4)]
        for s, val in _rhs_operands(b11, b12, b21, b22):
            _st(w, s * HD + i, val)

    def prep_proj_steps(w):
        return [P(prep_proj, w, i) for i in range(0, HD, 16)]

    def strassen_steps(lhs, w, pm, pn, emit):
        def product(ms, t, i, n):
            s = SLOTS[t]
            ms.append(_dot(_ld(lhs.at[t], i, i + pm), _ld(w, s * HD, (s + 1) * HD, slice(n, n + pn))))
            if t == 6:
                emit(i, n, *_combine(ms))
        steps = []
        for n in range(0, HD, pn):
            for i in range(0, HB, pm):
                ms = []
                steps += [P(product, ms, t, i, n) for t in range(7)]
        return steps

    def put_qkv(m, b, n, y):
        if m == 0:
            y = y * QSCALE
        rows = y.shape[0]
        for j in range(n // 128, (n + y.shape[1]) // 128):
            yj = y[:, j * 128 - n:(j + 1) * 128 - n]
            if m == 0:
                q_scr[j, b:b + rows, :] = yj
            elif m == 1:
                k_scr[j, HALO + b:HALO + b + rows, :] = yj
            else:
                v_scr[j][HALO + b:HALO + b + rows, :] = yj
                if b == 0:
                    v_scr[j][0:HALO, :] = jnp.broadcast_to(yj[0:1, :], (HALO, 128))

    def qkv(m, r):
        def emit(i, n, c11, c12, c21, c22):
            for di, dn, y in ((0, 0, c11), (0, HD, c12), (HB, 0, c21), (HB, HD, c22)):
                put_qkv(m, r * MB + i + di, n + dn, y)
        return strassen_steps(xa.at[r], wqkv_p[m], 128, 128, emit)

    def w_plain(m, k0, k1, n, pn):
        row = (1 + 2 * (n // HD)) * HD
        return _ld(wqkv_p[m], row + k0, row + k1, slice(n % HD, n % HD + pn))

    def proj_plain(m, i, n):
        put_qkv(m, i, n, _dot(_ld(xn0, i, i + 128), w_plain(m, 0, D, n, 128)))

    def probs_steps(r, half):
        base = r * MB + half * (MB // 2)
        items = [(b, w) for b in range(base, base + MB // 2, R) for w in range(W)]
        s1, s2, done, qs = {}, {}, [], {}

        def step(t):
            if t < len(items):
                b, w = items[t]
                if w == 0:
                    qs[b] = [q_scr[j, b:b + R, :] for j in range(8)]
                p = None
                for j in range(8):
                    u = qs[b][j] * k_scr[j, HALO + b - DIL * w:HALO + b - DIL * w + R, :]
                    p = u if p is None else p + u
                s1[t] = (p, pltpu.roll(p, 64, 1))
            if 0 <= t - DLY < len(items):
                u, v = s1.pop(t - DLY)
                u = u + v
                s2[t - DLY] = (u, pltpu.roll(u, 32, 1))
            if t - 2 * DLY >= 0:
                b, w = items[t - 2 * DLY]
                u, v = s2.pop(t - 2 * DLY)
                p = u + v
                if b < DIL * w:
                    pos = b + lax.broadcasted_iota(jnp.int32, (R, 128), 0)
                    p = jnp.where(pos >= DIL * w, p, -1e9 * LOG2E)
                done.append(p)
                if w == W - 1:
                    mx = functools.reduce(jnp.maximum, done)
                    es = [jnp.exp2(p - mx) for p in done]
                    inv = 1.0 / functools.reduce(lambda u, v: u + v, es)
                    for w in range(W):
                        q_scr[w, b:b + R, :] = es[w] * inv
                    done.clear()
        return [P(step, t) for t in range(len(items) + 2 * DLY)]

    def pv(b, j):
        o = None
        for w in range(W):
            t = q_scr[w, b:b + RP, :] * v_scr[j][HALO + b - DIL * w:HALO + b - DIL * w + RP, :]
            o = t if o is None else o + t
        return o

    def pv_steps(r):
        def step(os, i, j, di, dj):
            os.append(pv(r * MB + i + di, j + dj))
            if len(os) == 4:
                for t, val in enumerate(_lhs_operands(*os)):
                    _st(a_scr[r].at[t], i, val, slice(j * 128, (j + 1) * 128))
        steps = []
        for i in range(0, HB, RP):
            for j in range(4):
                os = []
                steps += [P(step, os, i, j, di, dj) for di in (0, HB) for dj in (0, 4)]
        return steps

    def load_x(r, b):
        x = io[r][b:b + RL, :].astype(F32)
        xs[r, b:b + RL, :] = x
        return x

    def ln_steps(r, from_input=False):
        def step(prev, b):
            ys = []
            for i in (b, HB + b):
                x = load_x(r, i) if from_input else xs[r, i:i + RL, :]
                if prev:
                    keep = jnp.full((RL, 128), flag[0], jnp.int32) == 1
                    x = jnp.concatenate([jnp.where(keep, x[:, :128], prev[0]), x[:, 128:]], axis=1)
                ys.append(_ln(x))
            top, bot = ys
            prev[:] = [bot[:, :128]]
            for t, val in enumerate(_lhs_operands(top[:, :HD], top[:, HD:], bot[:, :HD], bot[:, HD:])):
                _st(xa.at[r, t], b, val)
        prev = []
        return [P(step, prev, b) for b in range(0, HB, RL)]

    def ln_plain_steps(i0, i1):
        def step(b):
            _st(xn0, b, _ln(load_x(0, b)))
        return [P(step, b) for b in range(i0, i1, RL)]

    def wo_steps(r):
        def emit(i, n, c11, c12, c21, c22):
            for di, dn, y in ((0, 0, c11), (0, HD, c12), (HB, 0, c21), (HB, HD, c22)):
                xs[r, i + di:i + di + 128, n + dn:n + dn + 128] += y
        return strassen_steps(a_scr[r], wo_p, 128, 128, emit)

    def up_steps(p, r, slot, pm=HB, pn=128):
        def product(ms, hs, c, t, i, n):
            s = SLOTS[t]
            ms.append(_dot(_ld(xa.at[r, t], i, i + pm), wup[c, s * HD:(s + 1) * HD, n:n + pn]))
            if t == 6:
                gt, ut, gb, ub = _combine(ms)
                ms.clear()
                hs.append((_silu(gt) * ut, _silu(gb) * ub))
                if len(hs) == 2:
                    for u, val in enumerate(_lhs_operands(hs[0][0], hs[1][0], hs[0][1], hs[1][1])):
                        _st(ha.at[slot, u], i, val, slice(n, n + pn))
        steps = []
        for n in range(0, FC, pn):
            for i in range(0, HB, pm):
                ms, hs = [], []
                steps += [P(product, ms, hs, c, t, i, n) for c in (2 * p, 2 * p + 1) for t in range(7)]
        return steps

    def down_steps(p, r, slot, pm=HB, pn=128, i0=0, i1=HB):
        def product(ms, t, i, n):
            s = SLOTS[t]
            ms.append(_dot(_ld(ha.at[slot, t], i, i + pm), wdn[p, s * FC:(s + 1) * FC, n:n + pn]))
            if t == 6:
                for (di, dn), y in zip(((0, 0), (0, HD), (HB, 0), (HB, HD)), _combine(ms)):
                    xs[r, i + di:i + di + pm, n + dn:n + dn + pn] += y
        steps = []
        for n in range(0, HD, pn):
            for i in range(i0, i1, pm):
                ms = []
                steps += [P(product, ms, t, i, n) for t in range(7)]
        return steps

    flag[0] = 1
    queue = [cp_wq[0], cp_x0[0], cp_wq[1], cp_wq[2], cp_wq[3], cp_x0[1]] + cp_wk + [cp_wv]
    for c in queue[:4]:
        c.start()
    queue = queue[4:]

    def land(c):
        c.wait()
        if queue:
            queue.pop(0).start()

    k_scr[:, 0:HALO, :] = jnp.zeros((8, HALO, 128), F32)
    land(cp_wq[0])
    steps = permute_qkv_steps(0, [0])
    _merge(steps[:8])
    land(cp_x0[0])
    _merge(steps[8:], ln_plain_steps(0, HB))

    def q_slab(t, n):
        y = _dot(_ld(xn0, 0, HB, slice(t * 256, (t + 1) * 256)), w_plain(0, t * 256, (t + 1) * 256, n, 256))
        for j in range(n // 128, n // 128 + 2):
            yj = y[:, j * 128 - n:(j + 1) * 128 - n]
            if t:
                yj = q_scr[j, 0:HB, :] + yj
            q_scr[j, 0:HB, :] = yj * QSCALE if t == 3 else yj

    def layer(l):
        pend = []

        def run(name, main, *sides):
            pend.append((main, sides))
            if name in ('K1', 'K2', 'K3', 'O0', 'O1', 'O2', 'L0'):
                return
            work = list(pend)
            pend.clear()

            @pl.when(flag[0] == 1)
            def _():
                for m, sd in work:
                    _merge(m, *sd)

        def halves(steps):
            return steps[:len(steps) // 2], steps[len(steps) // 2:]

        def first(steps, *waits):
            if l:
                return []
            for c in waits:
                c.wait()
            return steps

        def preps(name):
            ps = [p for p, nm in enumerate(('K3', 'F0b', 'O3', 'F0d', 'K2', 'V2', 'V3')) if nm == name]
            return first([s for p in ps for s in prep_steps(p)], *[c for p in ps for c in cp_ffn[p]])

        pwo = halves(permute_wo_steps())
        pb = va = vb = []
        for r in range(NB):
            if r == 0:
                if l:
                    run('Q0', qkv(0, r), ln_steps(NB - 2))
                    run('K0', qkv(1, r), ln_steps(NB - 1))
                else:
                    for t in range(4):
                        land(cp_wq[t + 1] if t < 3 else cp_x0[1])
                        run('Q0a', [P(q_slab, t, n) for n in range(0, D, 256)],
                            permute_qkv_steps(0, [t + 1]) if t < 3 else ln_plain_steps(HB, MB))
                    for t in range(4):
                        land(cp_wk[t])
                        run('Q0b', [P(proj_plain, 0, i, n) for n in (256 * t, 256 * t + 128)
                                    for i in range(HB, MB, 128)], permute_qkv_steps(1, [t]))
                    for c in queue + [cp_x[1], cp_wo, cp_x[2], cp_x[3]]:
                        c.start()
                    k0 = halves([P(proj_plain, 1, i, n) for n in range(0, D, 128) for i in range(0, MB, 128)])
                    run('K0a', k0[0], prep_proj_steps(wqkv_p[0]), ln_steps(0))
                    run('K0b', k0[1], first(permute_qkv_steps(2) + prep_proj_steps(wqkv_p[2]), cp_wv))
                    for cps in cp_ffn:
                        for c in cps:
                            c.start()
            else:
                ln2 = ln_steps(r - 2) if r > 1 else []
                ln2 = halves(ln2)
                run('Q%d' % r, qkv(0, r), pb, first(pwo[0] + prep_proj_steps(wqkv_p[1]), cp_wo) if r == 1 else [])
                run('K%d' % r, qkv(1, r), va, ln2[0], preps('K%d' % r), first(pwo[1]) if r == 1 else [])
            pa, pb = probs_steps(r, 0), probs_steps(r, 1)
            nxt = first(ln_steps(r + 1, True), cp_x[r + 1]) if r + 1 < NB else []
            if r == 0:
                run('V0', qkv(2, r), pa, nxt)
            else:
                run('V%d' % r, qkv(2, r), vb, nxt, ln2[1], preps('V%d' % r),
                    first(prep_proj_steps(wo_p)) if r == 1 else [])
                run('O%d' % (r - 1), wo_steps(r - 1), pa)
            va, vb = halves(pv_steps(r))
        def up(p, r):
            return up_steps(p, r, r % 2)

        def down(p, r):
            return down_steps(p, r, r % 2)

        run('F0a', up(0, 0), pb)
        run('F0b', _zip(up(0, 1), down(0, 0)), va + vb, preps('F0b'))
        run('O3', wo_steps(NB - 1), ln_steps(NB - 2), preps('O3'))
        run('F0c', _zip(up(0, 2), down(0, 1)), ln_steps(NB - 1))
        run('F0d', _zip(up(0, 3), down(0, 2)) + down(0, 3), preps('F0d'))

        def body(it, carry):
            p, half = 1 + it // 2, it % 2
            ups = [up_steps(p, 2 * half + u, u) for u in range(2)]
            downs = [down_steps(p, 2 * half + u, u) for u in range(2)]
            _merge(ups[0] + _zip(ups[1], downs[0]) + downs[1])
            return carry
        lax.fori_loop(0, 2 * (NP - 2), body, 0)
        p = NP - 1
        if l == 0:
            run('L0', up(p, 0) + _zip(up(p, 1), down(p, 0)))
            run('L1', _zip(up(p, 2), down(p, 1)), ln_steps(0))
            run('L2', _zip(up(p, 3), down(p, 2)) + down(p, 3), ln_steps(1))
        else:
            def write(r, i, n):
                for i0 in (i, HB + i):
                    io[r][i0:i0 + n, :] = xs[r, i0:i0 + n, :].astype(BF16)
                    cp_out(r, i0, n).start()

            main = up(p, 0)
            for r in range(NB - 1):
                main += _zip(up(p, r + 1), down(p, r)) + [P(write, r, 0, HB)]
            for i in range(0, HB, 128):
                main += down_steps(p, NB - 1, 1, 128, 128, i, i + 128) + [P(write, NB - 1, i, 128)]
            run('L', main)

    layer(0)
    layer(1)
    for r in range(NB):
        cp_out(r, 0, MB).wait()


@jax.jit
def pallas_interleave_layers__sliding_local_dilated__glu_gated_swiglu__prompt_kernel(
    A_x: jax.Array,
    A_wqkv: jax.Array,
    A_wo: jax.Array,
    B_x: jax.Array,
    B_w1: jax.Array,
    B_w3: jax.Array,
    B_w2: jax.Array,
):
    del B_x
    B, S, D = A_x.shape
    F = B_w1.shape[1]
    NC = F // FC
    MB = S // NB
    x = A_x.reshape(S, D)
    anyspec = pl.BlockSpec(memory_space=pl.ANY)
    out = pl.pallas_call(
        _kernel,
        in_specs=[anyspec] * 6,
        out_specs=anyspec,
        out_shape=jax.ShapeDtypeStruct((S, D), A_x.dtype),
        scratch_shapes=[
            pltpu.VMEM((3, D, D), BF16), [pltpu.VMEM((7 * D // 4, D // 2), U32)] * 3,
            pltpu.VMEM((D, D), BF16), pltpu.VMEM((7 * D // 4, D // 2), U32),
            pltpu.VMEM((NC, 7 * D // 2, FC), BF16), pltpu.VMEM((NC // 2, 7 * FC, D // 2), BF16),
            [pltpu.VMEM(((H + 1) * PAD + 7, 128), U32)] * 2,
            pltpu.VMEM((8, S, 128), F32), pltpu.VMEM((8, S + HALO, 128), F32),
            [pltpu.VMEM((S + HALO, 128), F32)] * 8,
            [pltpu.VMEM((7, MB // 4, D // 2), U32)] * 2,
            pltpu.VMEM((NB, MB, D), F32), pltpu.VMEM((MB // 2, D), U32),
            pltpu.VMEM((NB, 7, MB // 4, D // 2), U32), [pltpu.VMEM((MB, D), BF16)] * NB,
            pltpu.VMEM((2, 7, MB // 4, FC), U32),
            pltpu.SemaphoreType.DMA((NB,)), pltpu.SemaphoreType.DMA((13,)), pltpu.SemaphoreType.DMA((NC // 2,)), pltpu.SemaphoreType.DMA((NB,)),
            pltpu.SMEM((1,), jnp.int32),
        ],
        compiler_params=pltpu.CompilerParams(vmem_limit_bytes=126 * 1024 * 1024),
    )(x, A_wqkv, A_wo, B_w1, B_w3, B_w2)
    return out.reshape(B, S, D)
```

```python
import functools
import math
import jax
import jax.numpy as jnp
from jax import lax
import jax.experimental.pallas as pl
import jax.experimental.pallas.tpu as pltpu

H, DH, W, DIL = 32, 32, 8, 2
EPS = 1e-5
NB = 4
FC = 256
HALO = 16
PAD = DH + 1
R, RP, RL = 8, 16, 32
PC = 256
DLY = 4
SLOTS = (0, 1, 3, 2, 4, 5, 6)
LOG2E = math.log2(math.e)
QSCALE = DH ** -0.5 * LOG2E
F32, BF16, U32 = jnp.float32, jnp.bfloat16, jnp.uint32


def _ln(x):
    m = jnp.mean(x, axis=-1, keepdims=True)
    c = x - m
    v = jnp.mean(c * c, axis=-1, keepdims=True)
    return c * lax.rsqrt(v + EPS)


def _silu(g):
    hg = 0.5 * g
    return hg * jnp.tanh(hg) + hg


def _dot(a, b):
    return jnp.dot(a, b, preferred_element_type=F32)


def _ld(ref, r0, r1, cols=slice(None)):
    return pltpu.bitcast(ref[r0 // 2:r1 // 2, cols], BF16)


def _st(ref, r0, val, cols=slice(None)):
    ref[r0 // 2:(r0 + val.shape[0]) // 2, cols] = pltpu.bitcast(val.astype(BF16), U32)


def _lhs_operands(a11, a12, a21, a22):
    return (a11 + a22, a21 + a22, a11, a22, a11 + a12, a21 - a11, a12 - a22)


def _rhs_operands(b11, b12, b21, b22):
    return ((0, b11 + b22), (2, b21 - b11), (3, b12 - b22), (5, b11 + b12), (6, b21 + b22))


ORDER = (0, 1, 3, 2, 4, 5, 6)


def _combine(acc, t, m):
    if t in (0, 1):
        acc[t] = m
    elif t == 3:
        m1, m2 = acc.pop(0), acc.pop(1)
        acc['c11'], acc['c22'] = m1 + m, m1 - m2
        yield 2, m2 + m
    elif t == 2:
        acc[2] = m
        acc['c22'] = acc['c22'] + m
    elif t == 4:
        acc['c11'] = acc['c11'] - m
        yield 1, acc.pop(2) + m
    elif t == 5:
        yield 3, acc.pop('c22') + m
    else:
        yield 0, acc.pop('c11') + m


def _zip(main, side):
    n, out = len(main), []
    for i, f in enumerate(main):
        out += [f] + side[len(side) * i // n:len(side) * (i + 1) // n]
    return out


def _merge(main, *sides):
    n = len(main)
    for i, f in enumerate(main):
        f()
        for s in sides:
            for g in s[len(s) * i // n:len(s) * (i + 1) // n]:
                g()


def _kernel(x_hbm, wqkv_hbm, wo_hbm, w1_hbm, w3_hbm, w2_hbm, o_hbm,
            wqkv_raw, wqkv_p, wo_raw, wo_p, wup, wdn, tr_scr, q_scr, k_scr,
            v_scr, a_scr, xs, xn0, xa, io, ha, sem_x, sem_w, sem_f, sem_o, flag):
    _, MB, D = xs.shape
    HB, HD = MB // 2, D // 2
    a_scr = [a_scr[r % 2] for r in range(NB)]
    NP = wdn.shape[0]
    P = functools.partial

    cp_x = {r: pltpu.make_async_copy(x_hbm.at[r * MB:(r + 1) * MB, :], io[r], sem_x.at[r]) for r in range(1, NB)}

    def cp_out(r, i, n):
        return pltpu.make_async_copy(io[r].at[i:i + n, :], o_hbm.at[r * MB + i:r * MB + i + n, :], sem_o.at[r])

    cp_wq, cp_wk = [[pltpu.make_async_copy(wqkv_hbm.at[t * 256:(t + 1) * 256, m * D:(m + 1) * D],
                                           wqkv_raw.at[m, t * 256:(t + 1) * 256, :], sem_w.at[4 * m + t])
                     for t in range(4)] for m in range(2)]
    cp_wv = pltpu.make_async_copy(wqkv_hbm.at[:, 2 * D:3 * D], wqkv_raw.at[2], sem_w.at[8])
    cp_x0 = [pltpu.make_async_copy(x_hbm.at[i * HB:(i + 1) * HB, :], io[0].at[i * HB:(i + 1) * HB, :],
                                   sem_w.at[11 + i]) for i in range(2)]
    cp_wo = pltpu.make_async_copy(wo_hbm, wo_raw, sem_w.at[9])
    cp_ffn = []
    for p in range(NP):
        cps = [(w.at[:, c * FC:(c + 1) * FC], wup.at[c, s * HD:(s + 2) * HD, :])
               for c in (2 * p, 2 * p + 1) for w, s in ((w1_hbm, 1), (w3_hbm, 3))]
        cps += [(w2_hbm.at[2 * p * FC:(2 * p + 2) * FC, n:n + HD], wdn.at[p, s * FC:(s + 2) * FC, :])
                for n, s in ((0, 1), (HD, 3))]
        cp_ffn.append([pltpu.make_async_copy(a, b, sem_f.at[p]) for a, b in cps])

    def prep(w, c, rows, i, n):
        b11, b21, b12, b22 = [w[c, s * rows + i:s * rows + i + 16, n:n + PC].astype(F32) for s in (1, 2, 3, 4)]
        for s, val in _rhs_operands(b11, b12, b21, b22):
            w[c, s * rows + i:s * rows + i + 16, n:n + PC] = val.astype(BF16)

    def prep_steps(p):
        return [P(prep, w, c, rows, i, n)
                for w, c, rows in ((wup, 2 * p, HD), (wup, 2 * p + 1, HD), (wdn, p, FC))
                for i in range(0, rows, 16) for n in range(0, w.shape[2], PC)]

    def stage(slot, i, val):
        for hh in range(4):
            h = 4 * i + hh
            tr_scr[slot][h * PAD:h * PAD + DH, :] = val[hh * DH:(hh + 1) * DH, :]

    def gather(slot, j):
        return jnp.concatenate([tr_scr[slot][pl.ds(4 * j + dd, H, stride=PAD), :] for dd in range(4)], axis=0)

    def qkv_in(m, t, i):
        blk = pltpu.bitcast(wqkv_raw[m, t * 256:(t + 1) * 256, i * 128:(i + 1) * 128], U32)
        stage(t % 2, i, blk.T)

    def qkv_out(m, t, j):
        row = (1 + t // 2 + 2 * (j // 4)) * (HD // 2) + (t % 2) * 128
        wqkv_p[m][row:row + 128, (j % 4) * 128:(j % 4 + 1) * 128] = gather(t % 2, j).T

    def permute_qkv_steps(m, ts=range(4)):
        return [P(f, m, t, i) for t in ts for f in (qkv_in, qkv_out) for i in range(8)]

    def wo_in(c, i):
        stage(c % 2, i, pltpu.bitcast(wo_raw[i * 128:(i + 1) * 128, c * 128:(c + 1) * 128].astype(F32), U32))

    def wo_out(c, j):
        _st(wo_p, (1 + 2 * (c // 4)) * HD + j * 128, pltpu.bitcast(gather(c % 2, j), F32),
            slice((c % 4) * 128, (c % 4 + 1) * 128))

    def permute_wo_steps():
        return [P(f, c, i) for c in range(8) for f in (wo_in, wo_out) for i in range(8)]

    def prep_proj(w, i, n):
        cols = slice(n, n + PC)
        b11, b21, b12, b22 = [_ld(w, s * HD + i, s * HD + i + 16, cols).astype(F32) for s in (1, 2, 3, 4)]
        for s, val in _rhs_operands(b11, b12, b21, b22):
            _st(w, s * HD + i, val, cols)

    def prep_proj_steps(w):
        return [P(prep_proj, w, i, n) for i in range(0, HD, 16) for n in range(0, HD, PC)]

    def strassen_steps(lhs, w, pm, pn, emit):
        def product(ms, t, i, n):
            s = SLOTS[t]
            m = _dot(_ld(lhs.at[t], i, i + pm), _ld(w, s * HD, (s + 1) * HD, slice(n, n + pn)))
            for quad, y in _combine(ms, t, m):
                emit(i + HB * (quad // 2), n + HD * (quad % 2), y)
        steps = []
        for n in range(0, HD, pn):
            for i in range(0, HB, pm):
                ms = {}
                steps += [P(product, ms, t, i, n) for t in ORDER]
        return steps

    def put_qkv(m, b, n, y):
        if m == 0:
            y = y * QSCALE
        rows = y.shape[0]
        for j in range(n // 128, (n + y.shape[1]) // 128):
            yj = y[:, j * 128 - n:(j + 1) * 128 - n]
            if m == 0:
                q_scr[j, b:b + rows, :] = yj
            elif m == 1:
                k_scr[j, HALO + b:HALO + b + rows, :] = yj
            else:
                v_scr[j][HALO + b:HALO + b + rows, :] = yj
                if b == 0:
                    v_scr[j][0:HALO, :] = jnp.broadcast_to(yj[0:1, :], (HALO, 128))

    def qkv(m, r):
        def emit(i, n, y):
            put_qkv(m, r * MB + i, n, y)
        return strassen_steps(xa.at[r], wqkv_p[m], 128, 128, emit)

    def w_plain(m, k0, k1, n, pn):
        row = (1 + 2 * (n // HD)) * HD
        return _ld(wqkv_p[m], row + k0, row + k1, slice(n % HD, n % HD + pn))

    def proj_plain(m, i, n):
        put_qkv(m, i, n, _dot(_ld(xn0, i, i + 128), w_plain(m, 0, D, n, 128)))

    def probs_steps(r, half):
        base = r * MB + half * (MB // 2)
        items = [(b, w) for b in range(base, base + MB // 2, R) for w in range(W)]
        s1, s2, done, qs = {}, {}, [], {}

        def step(t):
            if t < len(items):
                b, w = items[t]
                if w == 0:
                    qs[b] = [q_scr[j, b:b + R, :] for j in range(8)]
                p = None
                for j in range(8):
                    u = qs[b][j] * k_scr[j, HALO + b - DIL * w:HALO + b - DIL * w + R, :]
                    p = u if p is None else p + u
                s1[t] = (p, pltpu.roll(p, 64, 1))
            if 0 <= t - DLY < len(items):
                u, v = s1.pop(t - DLY)
                u = u + v
                s2[t - DLY] = (u, pltpu.roll(u, 32, 1))
            if t - 2 * DLY >= 0:
                b, w = items[t - 2 * DLY]
                u, v = s2.pop(t - 2 * DLY)
                p = u + v
                if b < DIL * w:
                    pos = b + lax.broadcasted_iota(jnp.int32, (R, 128), 0)
                    p = jnp.where(pos >= DIL * w, p, -1e9 * LOG2E)
                done.append(p)
                if w == W - 1:
                    mx = functools.reduce(jnp.maximum, done)
                    es = [jnp.exp2(p - mx) for p in done]
                    inv = 1.0 / functools.reduce(lambda u, v: u + v, es)
                    for w in range(W):
                        q_scr[w, b:b + R, :] = es[w] * inv
                    done.clear()
        return [P(step, t) for t in range(len(items) + 2 * DLY)]

    def pv(b, j):
        o = None
        for w in range(W):
            t = q_scr[w, b:b + RP, :] * v_scr[j][HALO + b - DIL * w:HALO + b - DIL * w + RP, :]
            o = t if o is None else o + t
        return o

    def pv_steps(r):
        def step(os, i, j, di, dj):
            os.append(pv(r * MB + i + di, j + dj))
            if len(os) == 4:
                for t, val in enumerate(_lhs_operands(*os)):
                    _st(a_scr[r].at[t], i, val, slice(j * 128, (j + 1) * 128))
        steps = []
        for j in range(4):
            for i in range(0, HB, RP):
                os = []
                steps += [P(step, os, i, j, di, dj) for di in (0, HB) for dj in (0, 4)]
        return steps

    def load_x(r, b):
        x = io[r][b:b + RL, :].astype(F32)
        xs[r, b:b + RL, :] = x
        return x

    def ln_steps(r, from_input=False):
        def stats(prev, st, i):
            x = load_x(r, i) if from_input else xs[r, i:i + RL, :]
            if prev:
                keep = jnp.full((RL, 128), flag[0], jnp.int32) == 1
                x = jnp.concatenate([jnp.where(keep, x[:, :128], prev[0]), x[:, 128:]], axis=1)
            m = jnp.mean(x, axis=-1, keepdims=True)
            c = x - m
            rs = lax.rsqrt(jnp.mean(c * c, axis=-1, keepdims=True) + EPS)
            st.append((jnp.broadcast_to(m, (RL, 128)), jnp.broadcast_to(rs, (RL, 128))))
            if len(st) == 2:
                prev[:] = [st[-1][1]]

        def emit(st, b, n):
            ys = [(xs[r, i:i + RL, c0:c0 + 128] - m) * rs
                  for i, (m, rs) in zip((b, HB + b), st) for c0 in (n, HD + n)]
            for t, val in enumerate(_lhs_operands(*ys)):
                _st(xa.at[r, t], b, val, slice(n, n + 128))

        prev, steps = [], []
        for b in range(0, HB, RL):
            st = []
            steps += [P(stats, prev, st, b), P(stats, prev, st, HB + b)]
            steps += [P(emit, st, b, n) for n in range(0, HD, 128)]
        return steps

    def ln_plain_steps(i0, i1):
        def step(b):
            _st(xn0, b, _ln(load_x(0, b)))
        return [P(step, b) for b in range(i0, i1, RL)]

    def wo_steps(r):
        def emit(i, n, y):
            xs[r, i:i + 128, n:n + 128] += y
        return strassen_steps(a_scr[r], wo_p, 128, 128, emit)

    def up_steps(p, r, slot, pm=HB, pn=256):
        def product(ms, hs, c, t, i, n):
            s = SLOTS[t]
            m = _dot(_ld(xa.at[r, t], i, i + pm), wup[c, s * HD:(s + 1) * HD, n:n + pn])
            for quad, y in _combine(ms, t, m):
                if quad in (1, 2):
                    ms['keep', quad] = y
                elif quad == 3:
                    hs.append(_silu(ms.pop(('keep', 2))) * y)
                else:
                    hs.append(_silu(y) * ms.pop(('keep', 1)))
            if len(hs) == 4:
                for u, val in enumerate(_lhs_operands(hs[1], hs[3], hs[0], hs[2])):
                    _st(ha.at[slot, u], i, val, slice(n, n + pn))
        steps = []
        for n in range(0, FC, pn):
            for i in range(0, HB, pm):
                ms, hs = {}, []
                steps += [P(product, ms, hs, c, t, i, n) for c in (2 * p, 2 * p + 1) for t in ORDER]
        return steps

    def down_steps(p, r, slot, pm=HB, pn=128, i0=0, i1=HB):
        def product(ms, t, i, n):
            s = SLOTS[t]
            m = _dot(_ld(ha.at[slot, t], i, i + pm), wdn[p, s * FC:(s + 1) * FC, n:n + pn])
            for quad, y in _combine(ms, t, m):
                i0, n0 = i + HB * (quad // 2), n + HD * (quad % 2)
                xs[r, i0:i0 + pm, n0:n0 + pn] += y
        steps = []
        for n in range(0, HD, pn):
            for i in range(i0, i1, pm):
                ms = {}
                steps += [P(product, ms, t, i, n) for t in ORDER]
        return steps

    flag[0] = 1
    queue = [cp_wq[0], cp_x0[0], cp_wq[1], cp_wq[2], cp_wq[3], cp_x0[1]] + cp_wk + [cp_wv]
    for c in queue[:4]:
        c.start()
    queue = queue[4:]

    def land(c):
        c.wait()
        if queue:
            queue.pop(0).start()

    k_scr[:, 0:HALO, :] = jnp.zeros((8, HALO, 128), F32)
    land(cp_wq[0])
    steps = permute_qkv_steps(0, [0])
    _merge(steps[:8])
    land(cp_x0[0])
    _merge(steps[8:], ln_plain_steps(0, HB))

    def q_slab(t, n):
        y = _dot(_ld(xn0, 0, HB, slice(t * 256, (t + 1) * 256)), w_plain(0, t * 256, (t + 1) * 256, n, 256))
        for j in range(n // 128, n // 128 + 2):
            yj = y[:, j * 128 - n:(j + 1) * 128 - n]
            if t:
                yj = q_scr[j, 0:HB, :] + yj
            q_scr[j, 0:HB, :] = yj * QSCALE if t == 3 else yj

    def layer(l):
        pend = []

        def run(name, main, *sides):
            pend.append((main, sides))
            if name in ('K1', 'K2', 'K3', 'O0', 'O1', 'O2', 'L0'):
                return
            work = list(pend)
            pend.clear()

            @pl.when(flag[0] == 1)
            def _():
                for m, sd in work:
                    _merge(m, *sd)

        def halves(steps):
            return steps[:len(steps) // 2], steps[len(steps) // 2:]

        def first(steps, *waits):
            if l:
                return []
            for c in waits:
                c.wait()
            return steps

        def preps(name):
            ps = [p for p, nm in enumerate(('K3', 'F0b', 'O3', 'F0d', 'K2', 'V2', 'V3')) if nm == name]
            return first([s for p in ps for s in prep_steps(p)], *[c for p in ps for c in cp_ffn[p]])

        pwo = halves(permute_wo_steps())
        pb = va = vb = []
        for r in range(NB):
            if r == 0:
                if l:
                    run('Q0', qkv(0, r), ln_steps(NB - 2))
                    run('K0', qkv(1, r), ln_steps(NB - 1))
                else:
                    for t in range(4):
                        land(cp_wq[t + 1] if t < 3 else cp_x0[1])
                        run('Q0a', [P(q_slab, t, n) for n in range(0, D, 256)],
                            permute_qkv_steps(0, [t + 1]) if t < 3 else ln_plain_steps(HB, MB))
                    for t in range(4):
                        land(cp_wk[t])
                        run('Q0b', [P(proj_plain, 0, i, n) for n in (256 * t, 256 * t + 128)
                                    for i in range(HB, MB, 128)], permute_qkv_steps(1, [t]))
                    for c in queue + [cp_x[1], cp_wo, cp_x[2], cp_x[3]]:
                        c.start()
                    k0 = halves([P(proj_plain, 1, i, n) for n in range(0, D, 128) for i in range(0, MB, 128)])
                    run('K0a', k0[0], prep_proj_steps(wqkv_p[0]), ln_steps(0))
                    run('K0b', k0[1], first(permute_qkv_steps(2) + prep_proj_steps(wqkv_p[2]), cp_wv))
                    for cps in cp_ffn:
                        for c in cps:
                            c.start()
            else:
                ln2 = halves(ln_steps(r - 2) if r > 1 else [])
                run('Q%d' % r, qkv(0, r), pb, first(pwo[0] + prep_proj_steps(wqkv_p[1]), cp_wo) if r == 1 else [])
                run('K%d' % r, qkv(1, r), va, ln2[0], preps('K%d' % r), first(pwo[1]) if r == 1 else [])
            pa, pb = probs_steps(r, 0), probs_steps(r, 1)
            nxt = first(ln_steps(r + 1, True), cp_x[r + 1]) if r + 1 < NB else []
            if r == 0:
                run('V0', qkv(2, r), pa, nxt)
            else:
                run('V%d' % r, qkv(2, r), vb, nxt, ln2[1], preps('V%d' % r),
                    first(prep_proj_steps(wo_p)) if r == 1 else [])
                run('O%d' % (r - 1), wo_steps(r - 1), pa)
            va, vb = halves(pv_steps(r))

        def up(p, r):
            return up_steps(p, r, r % 2)

        def down(p, r):
            return down_steps(p, r, r % 2)

        run('F0a', up(0, 0), pb)
        run('F0b', _zip(up(0, 1), down(0, 0)), va + vb, preps('F0b'))
        run('O3', wo_steps(NB - 1), ln_steps(NB - 2), preps('O3'))
        run('F0c', _zip(up(0, 2), down(0, 1)), ln_steps(NB - 1))
        run('F0d', _zip(up(0, 3), down(0, 2)) + down(0, 3), preps('F0d'))

        def body(it, carry):
            p, half = 1 + it // 2, it % 2
            ups = [up_steps(p, 2 * half + u, u) for u in range(2)]
            downs = [down_steps(p, 2 * half + u, u) for u in range(2)]
            _merge(ups[0] + _zip(ups[1], downs[0]) + downs[1])
            return carry
        lax.fori_loop(0, 2 * (NP - 2), body, 0)
        p = NP - 1
        if l == 0:
            run('L0', up(p, 0) + _zip(up(p, 1), down(p, 0)))
            run('L1', _zip(up(p, 2), down(p, 1)), ln_steps(0))
            run('L2', _zip(up(p, 3), down(p, 2)) + down(p, 3), ln_steps(1))
        else:
            def write(r, i, n):
                for i0 in (i, HB + i):
                    io[r][i0:i0 + n, :] = xs[r, i0:i0 + n, :].astype(BF16)
                    cp_out(r, i0, n).start()

            main = up(p, 0)
            for r in range(NB - 1):
                main += _zip(up(p, r + 1), down(p, r)) + [P(write, r, 0, HB)]
            for i in range(0, HB, 128):
                main += down_steps(p, NB - 1, 1, 128, 128, i, i + 128) + [P(write, NB - 1, i, 128)]
            run('L', main)

    layer(0)
    layer(1)
    for r in range(NB):
        cp_out(r, 0, MB).wait()


@jax.jit
def pallas_interleave_layers__sliding_local_dilated__glu_gated_swiglu__prompt_kernel(
    A_x: jax.Array,
    A_wqkv: jax.Array,
    A_wo: jax.Array,
    B_x: jax.Array,
    B_w1: jax.Array,
    B_w3: jax.Array,
    B_w2: jax.Array,
):
    del B_x
    B, S, D = A_x.shape
    F = B_w1.shape[1]
    NC = F // FC
    MB = S // NB
    x = A_x.reshape(S, D)
    anyspec = pl.BlockSpec(memory_space=pl.ANY)
    out = pl.pallas_call(
        _kernel,
        in_specs=[anyspec] * 6,
        out_specs=anyspec,
        out_shape=jax.ShapeDtypeStruct((S, D), A_x.dtype),
        scratch_shapes=[
            pltpu.VMEM((3, D, D), BF16), [pltpu.VMEM((7 * D // 4, D // 2), U32)] * 3,
            pltpu.VMEM((D, D), BF16), pltpu.VMEM((7 * D // 4, D // 2), U32),
            pltpu.VMEM((NC, 7 * D // 2, FC), BF16), pltpu.VMEM((NC // 2, 7 * FC, D // 2), BF16),
            [pltpu.VMEM(((H + 1) * PAD + 7, 128), U32)] * 2,
            pltpu.VMEM((8, S, 128), F32), pltpu.VMEM((8, S + HALO, 128), F32),
            [pltpu.VMEM((S + HALO, 128), F32)] * 8,
            [pltpu.VMEM((7, MB // 4, D // 2), U32)] * 2,
            pltpu.VMEM((NB, MB, D), F32), pltpu.VMEM((MB // 2, D), U32),
            pltpu.VMEM((NB, 7, MB // 4, D // 2), U32), [pltpu.VMEM((MB, D), BF16)] * NB,
            pltpu.VMEM((2, 7, MB // 4, FC), U32),
            pltpu.SemaphoreType.DMA((NB,)), pltpu.SemaphoreType.DMA((13,)), pltpu.SemaphoreType.DMA((NC // 2,)), pltpu.SemaphoreType.DMA((NB,)),
            pltpu.SMEM((1,), jnp.int32),
        ],
        compiler_params=pltpu.CompilerParams(vmem_limit_bytes=126 * 1024 * 1024),
    )(x, A_wqkv, A_wo, B_w1, B_w3, B_w2)
    return out.reshape(B, S, D)
```
